```python
import os as _os
_os.environ.setdefault("JAX_PLATFORMS", "cpu")
import jax
import jax.numpy as jnp

def _softmax(x, axis=-1):
    return jax.nn.softmax(x, axis=axis)
def _gelu(x):
    return jax.nn.gelu(x, approximate=True)
def _silu(x):
    return jax.nn.silu(x)
def _sigmoid(x):
    return jax.nn.sigmoid(x)
def _layernorm(x, axis=-1, eps=1e-5):
    m = jnp.mean(x, axis=axis, keepdims=True)
    v = jnp.var(x, axis=axis, keepdims=True)
    return (x - m) / jnp.sqrt(v + eps)
def _scatter_add(tgt, idx, src, axis=0):
    return tgt.at[idx].add(src)
def _segment_sum(src, seg, n):
    return jax.ops.segment_sum(src, seg, n)
class _Rng:
    def __init__(self, key):
        self._k = key
    def _next(self):
        self._k, sub = jax.random.split(self._k)
        return sub
    def normal(self, shape):
        return jax.random.normal(self._next(), shape, dtype=jnp.bfloat16)
    def randint(self, lo, hi, shape):
        return jax.random.randint(self._next(), shape, lo, hi, dtype=jnp.int32)
    def uniform(self, shape, lo=0.0, hi=1.0):
        return jax.random.uniform(self._next(), shape, jnp.bfloat16, lo, hi)
    def permutation(self, n):
        return jax.random.permutation(self._next(), n)


kernel_name = 'concat_heads__ssm_conv_s4__grouped_kv_mqa__prompt'

def setup_inputs():
    _rng = _Rng(jax.random.key(int.from_bytes(__import__("os").urandom(4), "little")))
    _w = (lambda a: (lambda t: t.astype(jnp.bfloat16) if jnp.issubdtype(t.dtype, jnp.floating) else t)(jnp.asarray(a)))
    def _A_setup():
        B, L, D, N = 1, 2048, 448, 256
        A_re = -jnp.exp((lambda *s: _rng.normal(s) * 0.1)(D, N))
        A_im = jnp.pi * (lambda *s: _rng.normal(s) * 0.1)(D, N)
        B_re = (lambda *s: _rng.normal(s) * 0.1)(D, N)
        B_im = (lambda *s: _rng.normal(s) * 0.1)(D, N)
        C_re = (lambda *s: _rng.normal(s) * 0.1)(D, N)
        C_im = (lambda *s: _rng.normal(s) * 0.1)(D, N)
        log_dt = (lambda *s: _rng.normal(s) * 0.1)(D) * 0.5 - 4.0
        Dskip = (lambda *s: _rng.normal(s) * 0.05)(D)
        return {
            "u": _w((lambda *s: _rng.normal(s) * 0.05)(B, L, D)),
            "A_re": _w(A_re),
            "A_im": _w(A_im),
            "B_re": _w(B_re),
            "B_im": _w(B_im),
            "C_re": _w(C_re),
            "C_im": _w(C_im),
            "log_dt": _w(log_dt),
            "Dskip": _w(Dskip),
        }
    _A_in = _A_setup()

    def _B_setup():
        B, S, D, H = 1, 2048, 448, 16
        Dh = D // H
        return {
            "x": _w((lambda *s: _rng.normal(s) * 0.05)(B, S, D)),
            "wq": _w((lambda *s: _rng.normal(s) * 0.8)(D, H * Dh)),
            "wk": _w((lambda *s: _rng.normal(s) * 0.8)(D, Dh)),
            "wv": _w((lambda *s: _rng.normal(s) * 0.05)(D, Dh)),
            "wo": _w((lambda *s: _rng.normal(s) * 0.05)(H * Dh, D)),
        }
    _B_in = _B_setup()

    return {
        "A_u": _A_in["u"],
        "A_A_re": _A_in["A_re"],
        "A_A_im": _A_in["A_im"],
        "A_B_re": _A_in["B_re"],
        "A_B_im": _A_in["B_im"],
        "A_C_re": _A_in["C_re"],
        "A_C_im": _A_in["C_im"],
        "A_log_dt": _A_in["log_dt"],
        "A_Dskip": _A_in["Dskip"],
        "B_x": _B_in["x"],
        "B_wq": _B_in["wq"],
        "B_wk": _B_in["wk"],
        "B_wv": _B_in["wv"],
        "B_wo": _B_in["wo"],
    }

def reference(A_u, A_A_re, A_A_im, A_B_re, A_B_im, A_C_re, A_C_im, A_log_dt, A_Dskip, B_x, B_wq, B_wk, B_wv, B_wo):
    def _A_ref(u, A_re, A_im, B_re, B_im, C_re, C_im, log_dt, Dskip):
        Bsz, L, D = u.shape
        dt = jnp.exp(log_dt)[:, None]
        A = A_re + 1j * A_im
        Bc = B_re + 1j * B_im
        Cc = C_re + 1j * C_im
        logdA = dt * A
        dB = dt * Bc
        l = (lambda x, dt: x.astype(dt))(jnp.arange(L), A_re.dtype)
        P = jnp.exp(logdA[:, :, None] * l[None, None, :])
        K = jnp.einsum("dn,dnl,dn->dl", Cc, P, dB).real
        L2 = 2 * L
        Kp = jnp.pad(K, ((0, 0), (0, L)))
        up = (lambda x, *d: x.transpose(*d))(u, 0, 2, 1)
        up = jnp.pad(up, ((0, 0), (0, 0), (0, L)))
        Kf = (lambda x, axes=(-2,-1): jnp.fft.rfft2(x.astype(jnp.float32), axes=axes))(Kp[:, None, :], axes=(-2, -1))
        Uf = (lambda x, axes=(-2,-1): jnp.fft.rfft2(x.astype(jnp.float32), axes=axes))(up[:, :, None, :], axes=(-2, -1))
        Yf = Uf * Kf[None, :, :, :]
        y = (lambda x, s, axes=(-2,-1): jnp.fft.irfft2(x, s=s, axes=axes).astype(jnp.bfloat16))(Yf, (1, L2), axes=(-2, -1))[:, :, 0, :L]
        y = (lambda x, *d: x.transpose(*d))(y, 0, 2, 1) + u * Dskip[None, None, :]
        return y

    def _B_ref(x, wq, wk, wv, wo):
        B, S, D = x.shape
        H = 16
        Dh = D // H
        q = (lambda x, *d: x.transpose(*d))((x @ wq).reshape(B, S, H, Dh), 0, 2, 1, 3)
        k = x @ wk
        v = x @ wv
        scores = jnp.einsum("bhqd,bkd->bhqk", q, k) * (Dh ** -0.5)
        p = _softmax(scores, axis=-1)
        o = jnp.einsum("bhqk,bkd->bhqd", p, v)
        return (lambda x, *d: x.transpose(*d))(o, 0, 2, 1, 3).reshape(B, S, H * Dh) @ wo

    a = _A_ref(A_u, A_A_re, A_A_im, A_B_re, A_B_im, A_C_re, A_C_im, A_log_dt, A_Dskip)
    b = _B_ref(B_x, B_wq, B_wk, B_wv, B_wo)
    return jnp.concatenate([a, b], axis=-1)
```

```python
import ml_dtypes
import numpy as np

import jax
import jax.numpy as jnp
from jax import lax
import jax.experimental.pallas as pl
import jax.experimental.pallas.tpu as pltpu

L = 2048
D = 448
N = 256
H = 16
DH = 28
W = 512
CH = 128
NCH = L // CH
T = 128
NB = L // T
GA = 4
GC = 5
POWERS_COST = 2
LAG_A = 3
LAG_C = 1
KORD = (0, 1, 2, 3, 4, 5, 6, 7)
KP_LAG = 3
PW = 1
DA, DB = 0, 4
UP = 4
Z0, Z1, Z2 = 4, 7, 12
LAG_P = 2
LAST_AT = (14, 18, 22, 26)
KP_AT = 4
PVF = 1
UN = 1
PEEL = 2
NO = 14
OP = 15
OL = 3
QP = 1
NQ = 54
NU = 8
PST = 9
CONV_STEP = 2
BCAST = 1
KBF = 0
F32 = jnp.float32
BF16 = jnp.bfloat16
U32 = jnp.uint32
NT_DIMS = (((1,), (1,)), ((), ()))

HI = (1, 2, 3, 4, 258, 260, 516, 772)
LO = tuple(4 * a for a in range(64)) + tuple(1028 + 8 * b for b in range(32))
POWER_PLAN = (
    ("x", 0, 1), ("z", 1, 1), ("x", 0, 2), ("x", 1, 2), ("x", 2, 2), ("z", 2, 2), ("z", 4, 4), ("z", 8, 4), ("z", 8, 8),
    ("z", 16, 4), ("z", 16, 12), ("z", 16, 8), ("z", 16, 16), ("z", 32, 8), ("z", 32, 16), ("z", 32, 24),
    ("z", 32, 32), ("z", 64, 32), ("z", 64, 64), ("z", 128, 32), ("z", 128, 96), ("z", 128, 64), ("z", 128, 128),
    ("x", 2, 256), ("x", 4, 256), ("z", 256, 256), ("x", 4, 512), ("x", 260, 512), ("z", 512, 512),
    ("z", 1024, 4), ("z", 1028, 64), ("z", 1028, 128), ("z", 1028, 192))
T_OF_BLOCK = (0, 1, 2, 3, 4, 5, 6, 7, 8, 9, 10, 11, 12, 5, 13, 7)
M_OF_BLOCK = (0, 1, 2, 3, 4, 5, 4, 5, 6, 7, 8, 7, 8, 7, 8, 7)


def _pack_np(a):
    bits = a.astype(np.float32).astype(ml_dtypes.bfloat16).view(np.uint16).astype(np.uint32)
    return bits[..., 0::2, :] | (bits[..., 1::2, :] << 16)


def _pack(a):
    return pltpu.bitcast(a.astype(BF16), jnp.uint32)


def _unpack(a):
    return pltpu.bitcast(a, BF16)


def _constants():
    f = np.arange(64)
    theta = np.pi * (2 * f + 1) / 256.0
    theta = np.concatenate([theta, -(np.pi * (2 * (127 - f) + 1) / 256.0)])

    def fwd(pos):
        ang = np.asarray(pos, np.float64)[:, None] * theta[None, :]
        return np.concatenate([np.cos(ang), -np.sin(ang)], axis=1)

    lane = np.arange(128)
    rows = [np.array([h + lo for lo in LO] + [-1] * 32) for h in HI]
    x01 = np.where(lane < 64, rows[0], np.roll(rows[1], 64))
    x23 = np.where(lane < 64, rows[2], np.roll(rows[3], 64))
    t2 = np.where(lane < 64, rows[4], np.roll(rows[5], 64))
    packed = [
        np.where((lane & 32) == 0, x01, np.roll(x23, 32)),
        np.where((lane & 32) != 0, x01, np.roll(x23, 96)),
        np.where(lane == 63, rows[3], t2), t2,
        np.where(lane == 63, rows[5], rows[6]), rows[6],
        np.where(lane == 63, rows[6], rows[7]), rows[7],
        np.where(lane == 63, rows[7], rows[3]), rows[3],
        np.where(lane == 95, rows[3], rows[5]), rows[5],
        np.where(lane == 95, rows[5], rows[6]),
        np.where(lane == 95, rows[6], rows[7]),
    ]
    lag_bf16 = np.arange(L + 1).astype(np.float32).astype(ml_dtypes.bfloat16).astype(np.int64)
    mats = {}
    for blk in range(NB):
        held = packed[T_OF_BLOCK[blk]]
        m = np.zeros((128, 256))
        for r in range(1, T + 1):
            (src,) = np.nonzero(held == lag_bf16[T * blk + r])
            m[src[0]] += fwd([r])[0]
        prev = mats.setdefault(M_OF_BLOCK[blk], m)
        assert np.array_equal(prev, m)
    fw = np.stack([mats[i] for i in range(9)] + [fwd(np.arange(T))])
    inv = []
    for par in range(2):
        ang = (2 * np.arange(64) + par)[:, None] * theta[None, :64]
        inv.append(np.concatenate([np.cos(ang), -np.sin(ang)], axis=1) / 128.0)
    return _pack_np(fw), _pack_np(np.stack(inv))


_FWD, _INV = _constants()


def _cmul(a, b):
    return a[0] * b[0] - a[1] * b[1], a[0] * b[1] + a[1] * b[0]


def _token(*values):
    tok = None
    for v in values:
        v = pltpu.bitcast(v, U32)
        for r in range(0, v.shape[0], 8):
            for c in range(0, v.shape[1], 128):
                tile = v[r:r + 8, c:c + 128]
                tok = tile if tok is None else tok | tile
    return tok


def chain(*gens):
    for gen in gens:
        yield from gen


def _kernel(u_hbm, are_hbm, aim_hbm, bre_hbm, bim_hbm, cre_hbm, cim_hbm, ldt_hbm, dsk_hbm,
            x_hbm, wq_hbm, wk_hbm, wv_hbm, wo_hbm, fw_hbm, inv_hbm,
            out_hbm,
            u_v, par_v, ldt_v, dsk_v, x_v, wq_v, wk_v, wv_v, wo_v, fw_v, inv_v, out_v,
            wt, wot, qt, kc, vtc, s_buf, ot, dtc, k0c, z1, pw, mul, kbuf, tbuf, hlast, gbuf, ubuf, ybuf, yst, zero_ref,
            x_sem, u_sem, in_sem, out_sem):
    def x_cp(i):
        tok = pl.ds(i * T if isinstance(i, int) else pl.multiple_of(i * T, T), T)
        return pltpu.make_async_copy(x_hbm.at[0, :, tok], x_v.at[i], x_sem.at[i])

    def u_cp(i):
        rows = pl.ds(i * 32 if isinstance(i, int) else pl.multiple_of(i * 32, 32), 32)
        return pltpu.make_async_copy(u_hbm.at[0, rows], u_v.at[rows], u_sem.at[i])

    pairs = [(r, par_v.at[i]) for i, r in enumerate((are_hbm, aim_hbm, bre_hbm, bim_hbm, cre_hbm, cim_hbm))]
    pairs += [(ldt_hbm, ldt_v), (dsk_hbm, dsk_v), (wq_hbm, wq_v), (wk_hbm, wk_v), (wv_hbm, wv_v),
              (fw_hbm.at[9], fw_v.at[9]), (fw_hbm.at[pl.ds(0, 9)], fw_v.at[pl.ds(0, 9)]), (wo_hbm, wo_v), (inv_hbm, inv_v)]
    cps = [pltpu.make_async_copy(src, dst, in_sem.at[i]) for i, (src, dst) in enumerate(pairs)]
    first_cp, weight_cp, second_cp, late_cp = [cps[6]] + cps[:2], cps[8:11], cps[2:6] + [cps[7], cps[11]], cps[12:]
    for cp in first_cp + weight_cp + [x_cp(i) for i in range(4)]:
        cp.start()

    def pad_rows(a, rows):
        return jnp.concatenate([a, jnp.zeros((rows - a.shape[0], a.shape[1]), a.dtype)], axis=0)

    def transpose_weight(w_ref, dst):
        for j in range(4):
            wd = min(128, D - 128 * j)
            panel = w_ref[:, 128 * j:128 * j + wd].astype(F32)
            if wd < 128:
                panel = jnp.concatenate([panel, jnp.zeros((D, 128 - wd), F32)], axis=1)
            dst[64 * j:64 * j + wd // 2, :] = _pack(pad_rows(panel, 512).T[:wd, :D])

    def to_column(row):
        row = jnp.concatenate([row, jnp.zeros((1, 512 - D), F32)], axis=1)
        return jnp.broadcast_to(row, (128, 512)).T

    def tie(words, tokens):
        if not tokens:
            return words
        zero = zero_ref[...]
        rows = [words[r:r + 8] for r in range(0, words.shape[0], 8)]
        for i, tok in enumerate(tokens):
            r = max((i + 1) * len(rows) // len(tokens) - 1, 0)
            first = rows[r][:, :128] | (tok & zero)
            rows[r] = first if words.shape[1] == 128 else jnp.concatenate([first, rows[r][:, 128:]], axis=1)
        return jnp.concatenate(rows, axis=0)

    def project_q(blk, tokens=()):
        qt[blk] = jnp.dot(_unpack(tie(wt[:D // 2, :], tokens)), x_v[blk], preferred_element_type=F32)

    def project_kv(i):
        tok = pl.ds(pl.multiple_of(i * W, W), W)
        x_t = jnp.concatenate([x_v[4 * i + j] for j in range(4)], axis=1)
        pr = jnp.dot(_unpack(wt[D // 2:, :]), x_t, preferred_element_type=F32)
        k_t, v_t = pr[:32], pr[32:]
        row32 = lax.broadcasted_iota(jnp.int32, (32, W), 0)
        k_both = pad_rows(jnp.concatenate([k_t, pltpu.roll(k_t, 4, 0)], axis=0), 128).T
        kc[pl.ds(pl.multiple_of(i * (W // 2), W // 2), W // 2), :] = _pack(k_both)
        for par in range(2):
            v_p = v_t if par == 0 else pltpu.roll(v_t, 4, 0)
            vtc[par, :, tok] = _pack(jnp.where(row32 == (DH if par == 0 else 0), 1.0, v_p))

    def q_window(pair, par):
        start = pl.multiple_of((pair % 8) * 56 + 24 * par, 8)
        q = jnp.concatenate([qt[4 * (pair // 8) + j, pl.ds(start, 32), :] for j in range(4)], axis=1)
        q = (q * np.float32(DH ** -0.5 * np.log2(np.e))).astype(BF16)
        zero = jnp.zeros((32, W), BF16)
        return jnp.concatenate([q, zero] if par == 0 else [zero, q], axis=0)

    def step(q_next, par_cur, mx_cur, fill, pending, pv_first=False):
        state = {}

        def scores(c, due):
            k_c = tie(kc[c * CH // 2:(c + 1) * CH // 2, :], due)
            s = jnp.dot(_unpack(k_c)[:, :64], q_next, preferred_element_type=F32)
            s_buf[c * CH:(c + 1) * CH, :] = s
            t = jnp.max(s.reshape(CH // 8, 8, W), axis=0)
            state["max"] = jnp.maximum(state["max"], t) if c else t

        def values(c, p, due):
            v_t = tie(vtc[par_cur, :, c * CH:(c + 1) * CH], due)
            o = jnp.dot(_unpack(v_t), p, preferred_element_type=F32)
            state["acc"] = state["acc"] + o if c else o

        if par_cur is not None:
            row_max = jnp.broadcast_to(jnp.max(mx_cur, axis=0, keepdims=True), (8, W))
        for c in range(NCH):
            due = pending.pop(0)
            if par_cur is None:
                scores(c, due)
            else:
                z = s_buf[c * CH:(c + 1) * CH, :].reshape(CH // 8, 8, W) - row_max[None]
                p = jnp.exp2(z).reshape(CH, W).astype(BF16)
                if q_next is None:
                    values(c, p, due)
                elif pv_first and c == NCH - 1:
                    values(c, p, [])
                    scores(c, due)
                else:
                    scores(c, due)
                    values(c, p, [])
            pending.append(fill(c))
        return state.get("max"), state.get("acc")

    def head_pair(pair, m, fill, lag=2, last=False):
        pending = [[]] * lag
        m, even = step(q_window(pair, 1), 0, m, fill, pending)
        m, odd = step(None if last else q_window(pair + 1, 0), 1, m, lambda c: fill(NCH + c), pending,
                      PVF)
        even = even * (1.0 / even[DH:DH + 1])
        odd = odd * (1.0 / odd[0:1])
        mid = jnp.where(lax.broadcasted_iota(jnp.int32, (8, W), 0) < 4, even[24:32], odd[0:8])
        rows = pl.ds(pl.multiple_of((pair % 8) * 56, 8), 56)
        o_t = jnp.concatenate([even[:24], mid, odd[8:]], axis=0)
        for j in range(4):
            ot[4 * (pair // 8) + j, rows, :] = o_t[:, j * T:(j + 1) * T]
        return m

    def out_features(blk, lo, hi, tokens=()):
        return jnp.dot(_unpack(tie(wot[:, lo:hi], tokens)), ot[blk, lo:hi, :].astype(BF16), preferred_element_type=F32)

    def put_out(blk, r):
        r = jnp.concatenate([jnp.zeros((64, T), F32), r], axis=0).T.astype(BF16)
        rows = pl.ds(blk * T if isinstance(blk, int) else pl.multiple_of(blk * T, T), T)
        out_v[rows, D:512] = r[:, 64:128]
        out_v[rows, 512:] = r[:, 128:]
        return _token(r)

    def discretize(g):
        rows = pl.ds(g * 8 if isinstance(g, int) else pl.multiple_of(g * 8, 8), 8)
        dt = dtc[0, rows, :]
        for lanes in (slice(0, 128), slice(128, 256)):
            mag = jnp.exp(dt * par_v[0, rows, lanes].astype(F32))
            ang = dt * par_v[1, rows, lanes].astype(F32)
            re, im = mag * jnp.cos(ang), mag * jnp.sin(ang)
            z1[0, rows, lanes], z1[1, rows, lanes] = re, im
            yield _token(re, im)

    def modes(first, count):
        return chain(*(discretize(first + j) for j in range(count)))

    def powers(g, slot):
        n = 8 * PW
        rows = pl.ds(pl.multiple_of(g * 8, n), n)
        dt = dtc[0, rows, :]
        dt = jnp.concatenate([dt, dt], axis=1)
        b_re, b_im, c_re, c_im = (par_v[i, rows, :].astype(F32) for i in range(2, 6))
        w = _cmul((c_re, c_im), (dt * b_re, dt * b_im))
        k0c[rows, :] = jnp.sum(w[0], axis=1, keepdims=True) + dtc[1, rows, :]
        yield _token(w[1])
        z = {0: (jnp.ones((n, N), F32), jnp.zeros((n, N), F32)), 1: (z1[0, rows, :], z1[1, rows, :])}

        def tiles(v):
            return [(j, part, half, v[part][8 * j:8 * j + 8, 128 * half:128 * (half + 1)])
                    for j in range(PW) for part in range(2) for half in range(2)]

        def put_strided(i, s, v):
            for j, part, half, tile in tiles(v):
                pw[slot + j, 4 * i + 2 * part + half, pl.ds(s, 8, stride=PST), :] = tile

        def put(p):
            if p in LO[8::8]:
                for j, part, half, tile in tiles(z[p]):
                    mul[slot + j, 4 * LO[8::8].index(p) + 2 * half + part] = tile
            if p < 32 and p % 4 == 0:
                put_strided(0, p // 4, z[p])
            if p < 64 and p % 8 == 0:
                put_strided(1, p // 8, z[p])

        put(0)
        x = {0: w}
        for kind, p, q in POWER_PLAN:
            if kind == "x":
                x[p + q] = _cmul(x[p], z[q])
                put_strided(2, HI.index(p + q), (x[p + q][0], -x[p + q][1]))
                yield _token(x[p + q][1])
                continue
            re, im = z[p]
            z[p + q] = (re * re - im * im, 2.0 * (re * im)) if p == q else _cmul(z[p], z[q])
            put(p + q)
            yield _token(z[p + q][0])

    def kernel_channel(g, j, slot, c):
        rows = slice(PST * c, PST * c + 8)
        taps = None
        for half in range(2):
            step4, step8, lhs = ([pw[slot, 4 * i + 2 * part + half, rows, :] for part in range(2)] for i in range(3))
            grp = [step4]
            for i in range(11):
                if BCAST:
                    m_i = [mul[slot, 4 * i + 2 * half + part, pl.ds(c, 8, stride=0), :] for part in range(2)]
                else:
                    m_i = [jnp.broadcast_to(mul[slot, 4 * i + 2 * half + part, c:c + 1, :], (8, 128)) for part in range(2)]
                grp.append(_cmul(step4 if i < 7 else step8, m_i))
            rhs = jnp.concatenate([jnp.concatenate([v[part] for v in grp], axis=0) for part in range(2)], axis=1)
            rhs, lhs = pad_rows(rhs, 128), jnp.concatenate(lhs, axis=1)
            if KBF:
                rhs = rhs.astype(BF16)
            if KBF > 1:
                lhs = pad_rows(lhs, 16).astype(BF16)
            t = lax.dot_general(lhs, rhs, NT_DIMS, preferred_element_type=F32)[:8]
            taps = t if taps is None else taps + t
        kbuf[g // 4, PST * (8 * j + c):PST * (8 * j + c) + 8, :] = taps

    def pack_taps(i):
        lane = lax.broadcasted_iota(jnp.int32, (32, 128), 1)
        r = [kbuf[i, pl.ds(j, 32, stride=PST), :] for j in range(8)]
        x01 = jnp.where(lane < 64, r[0], pltpu.roll(r[1], 64, 1))
        x23 = jnp.where(lane < 64, r[2], pltpu.roll(r[3], 64, 1))
        t2 = jnp.where(lane < 64, r[4], pltpu.roll(r[5], 64, 1))
        packed = [
            jnp.where((lane & 32) == 0, x01, pltpu.roll(x23, 32, 1)),
            jnp.where((lane & 32) != 0, x01, pltpu.roll(x23, 96, 1)),
            jnp.where(lane == 63, r[3], t2), t2,
            jnp.where(lane == 63, r[5], r[6]), r[6],
            jnp.where(lane == 63, r[6], r[7]), r[7],
            jnp.where(lane == 63, r[7], r[3]), r[3],
            jnp.where(lane == 95, r[3], r[5]), r[5],
            jnp.where(lane == 95, r[5], r[6]),
            jnp.where(lane == 95, r[6], r[7]),
        ]
        for blk in range(NB):
            tbuf[blk, pl.ds(pl.multiple_of(i * 16, 16), 16), :] = _pack(packed[T_OF_BLOCK[blk]])
        return _token(packed[0], packed[1], packed[2])

    def taps_dft(blk, slot):
        mat = jnp.where(blk < 6, blk, jnp.where(blk < 8, blk - 2, jnp.where(blk == 8, 6, 8 - blk % 2)))
        h = jnp.dot(_unpack(tbuf[blk]), _unpack(fw_v[mat]), preferred_element_type=F32)
        h_re, h_im = h[:, :128], h[:, 128:]
        g_re, g_im = h_re + hlast[1 - slot, 0], h_im + hlast[1 - slot, 1]
        even = (lax.broadcasted_iota(jnp.int32, (D, 128), 1) & 1) == 0
        hlast[slot, 0] = jnp.where(even, -1.0, 1.0) * h_im
        hlast[slot, 1] = jnp.where(even, 1.0, -1.0) * h_re
        g_dif, g_sum = g_im - g_re, g_re + g_im
        for t, v in enumerate((g_re, g_dif, g_sum)):
            gbuf[:, 3 * blk + t] = v.reshape(D // 8, 8, 128)

    def input_dft(g, b0, nb, tokens):
        rows = pl.ds(pl.multiple_of(g * 8, 8 * GA), 8 * GA)
        u_t = jnp.concatenate([u_v[rows, b * T:(b + 1) * T] for b in range(b0, b0 + nb)], axis=0)
        r = jnp.dot(_unpack(tie(_pack(u_t), tokens)), _unpack(fw_v[9]), preferred_element_type=F32)
        for b in range(nb):
            u_re, u_im = r[8 * GA * b:8 * GA * (b + 1), :128], r[8 * GA * b:8 * GA * (b + 1), 128:]
            for t, v in enumerate((u_re + u_im, u_re, u_im)):
                ubuf[pl.ds(g, GA), 3 * (b0 + b) + t] = v.reshape(GA, 8, 128)

    def block_conv(g, k):
        rows = pl.ds(pl.multiple_of(g * 8, 8), 8)
        low = lax.broadcasted_iota(jnp.int32, (8, 128), 1) < 64
        acc, loaded = {}, {}

        def g_at(d, t):
            if (d, t) not in loaded:
                loaded[d, t] = gbuf[g, 3 * d + t]
            return loaded[d, t]

        for j in range(2 * k + 2):
            if j and j % CONV_STEP == 0:
                yield _token(acc[2 * k + 1][2])
            u_j = [ubuf[g, 3 * j + t] for t in range(3)]
            for i in range(max(j, 2 * k), 2 * k + 2):
                prod = [g_at(i - j, t) * u_j[t] for t in range(3)]
                acc[i] = [a + b for a, b in zip(acc[i], prod)] if i in acc else prod
        done = []
        for i, (k1, k2, k3) in acc.items():
            y_re, y_im = k1 - k3, k1 + k2
            swapped = pltpu.roll(jnp.where(low, y_im, y_re), 64, 1)
            first = jnp.where(low, y_re, swapped)
            second = jnp.where(low, swapped, y_im)
            done += [first + second, first - second]
            ybuf[i, 0, rows, :], ybuf[i, 1, rows, :] = done[-2:]
        yield _token(*done)

    def inverse_dft(blk, slot):
        for par in range(2):
            y = lax.dot_general(_unpack(inv_v[par]), pad_rows(ybuf[blk, par], 512).astype(BF16), NT_DIMS,
                                preferred_element_type=F32)
            for j in range(4):
                yst[slot, j, pl.ds(par, 64, stride=2), :] = y[:, 128 * j:128 * (j + 1)]
        rows = pl.ds(blk * T, T)
        for j in range(4):
            wd = min(128, D - 128 * j)
            out_v[rows, 128 * j:128 * j + wd] = yst[slot, j].astype(BF16)[:, :wd]

    zero_ref[...] = jnp.zeros((8, 128), U32)
    for cp in first_cp:
        cp.wait()
    dtc[0] = to_column(jnp.exp(ldt_v[...].astype(F32).reshape(1, D)).astype(BF16).astype(F32))
    for cp in [x_cp(i) for i in range(4, NB)]:
        cp.start()

    @pl.loop(0, 4)
    def _(i):
        list(modes(Z0 * i, Z0))

    kbuf[0] = jnp.zeros(kbuf.shape[1:], F32)
    for cp in weight_cp:
        cp.wait()
    for i, w_ref in enumerate((wk_v, wv_v)):
        wt[D // 2 + 16 * i:D // 2 + 16 * (i + 1), :] = _pack(pad_rows(w_ref[...].astype(F32), 32))
    transpose_weight(wq_v, wt)

    def prologue(i, carry):
        for j in range(4):
            x_cp(4 * i + j).wait()
        project_kv(i)
        project_q(i, list(modes(4 * Z0 + Z1 * i, Z1)))
        return carry

    for cp in second_cp:
        cp.start()
    lax.fori_loop(0, 4, prologue, 0)
    early = list(modes(4 * (Z0 + Z1), Z2))
    m, _ = step(q_window(0, 0), None, None,
                lambda c: early[c * 2 * Z2 // (NCH - 2):(c + 1) * 2 * Z2 // (NCH - 2)], [[], []])
    for cp in second_cp:
        cp.wait()
    for cp in [u_cp(i) for i in range(D // 32)] + late_cp:
        cp.start()
    dtc[1] = to_column(dsk_v[...].astype(F32).reshape(1, D))

    def spread(streams, lag=2):
        span = 2 * NCH - lag

        def fill(c):
            out = []
            for gen, count in streams:
                count = span if count is None else count
                if c < span:
                    out += [next(gen) for _ in range((c + 1) * count // span - c * count // span)]
                if c == span - 1 and count != span:
                    assert next(gen, fill) is fill
            return [t for t in out if t is not None]
        return fill

    def once(job, at, lag=0):
        def gen():
            yield from [None] * at
            done = job()
            yield from [None] * lag + [done] + [None] * (2 * NCH)
        return gen(), None

    def loop(lo, hi, body, m):
        def unrolled(i, m):
            for j in range(UN):
                m = body(lo + UN * i + j, m)
            return m
        return lax.fori_loop(0, (hi - lo) // UN, unrolled, m)

    last_group = D // 8 - 1
    n_a = -(-(D // 8) // GA)
    n_c = -(-(D // 8) // GC)

    def phase_p(it, m):
        ahead = chain(*(powers(2 * it + j, 2 * it + j) for j in range(2)))
        n = (D // 8 - 4 * (Z0 + Z1) - Z2) // 2
        streams = [(ahead, 2 * (1 + len(POWER_PLAN))), (modes(D // 8 - n * (2 - it), n), 2 * n)]
        return head_pair(it, m, spread(streams, LAG_P), LAG_P)

    m = lax.fori_loop(0, 2, phase_p, m)

    def phase_a(it, m, query=True, more=True):
        u_cp(it).wait()
        cur, nxt = (it % 2) * GA, (1 - it % 2) * GA
        taps = (kernel_channel(GA * it + j, j, cur + j, c) for j in range(GA) for c in range(8))
        ahead = chain(*(powers(jnp.minimum(GA * (it + 1) + j, D // 8 - PW), nxt + j) for j in range(0, GA, PW)))

        def take(n):
            return [next(ahead) for _ in range(n if more else 0)]

        n_tok = (1 + len(POWER_PLAN)) * GA // PW - UP * NU
        streams = [once(lambda: pack_taps(jnp.maximum(it - 1, 0)), KP_AT, KP_LAG)]
        if query:
            streams.append(once(lambda: project_q(jnp.minimum(4 + it, NB - 1), take(NQ)), QP))
        streams += [(taps, 8 * GA), ((input_dft(GA * it, b, NB // UP, take(NU)) for b in range(0, NB, NB // UP)), UP)]
        if more:
            streams.append((ahead, n_tok - (NQ if query else 0)))
        m = head_pair(2 + it, m, spread(streams, LAG_A), LAG_A)
        return m

    m = loop(0, n_a - PEEL, phase_a, m)
    for it in range(n_a - PEEL, n_a):
        m = phase_a(jnp.int32(it), m, query=False, more=it + 1 < n_a)
    for cp in late_cp:
        cp.wait()
    pack_taps(n_a - 1)
    hlast[1, 0] = k0c[...]
    hlast[1, 1] = jnp.zeros((D, 128), F32)
    transpose_weight(wo_v, wot)

    def phase_b(it, m):
        return head_pair(16 + it, m, spread([((taps_dft(8 * it + j, j % 2) for j in range(8)), 8)]))

    m = lax.fori_loop(0, 2, phase_b, m)

    def phase_c(it, m):
        convs = chain(*(block_conv(jnp.minimum(GC * it + j, last_group), k)
                        for j in range(GC) for k in KORD))
        count = GC * sum(1 + (2 * k + 1) // CONV_STEP for k in range(8))
        proj = once(lambda: put_out(it, out_features(it, 0, D, [next(convs) for _ in range(NO)])), OP, OL)
        return head_pair(18 + it, m, spread([proj, (convs, count - NO)], LAG_C), LAG_C)

    m = loop(0, n_c, phase_c, m)

    def out_cp(i, rows, cols):
        return pltpu.make_async_copy(out_v.at[rows, cols], out_hbm.at[0, rows, cols], out_sem.at[i])

    done_cp = [out_cp(0, pl.ds(0, 3 * W), pl.ds(512, 384))]
    done_cp[0].start()
    m = head_pair(30, m, spread([((inverse_dft(blk, blk % 2) for blk in range(NB)), NB)]))
    done_cp += [out_cp(1, pl.ds(0, 3 * W), pl.ds(0, 512)), out_cp(2, pl.ds(3 * W, W), pl.ds(0, 384))]
    for cp in done_cp[1:]:
        cp.start()

    def fill_last(c):
        if c in LAST_AT:
            j = LAST_AT.index(c)
            qt[j] = out_features(12 + j, 0, 384)
        return []

    head_pair(31, m, fill_last, last=True)
    tails = [qt[j] + out_features(12 + j, 384, D) for j in range(W // T)]
    for j, r in enumerate(tails):
        put_out(12 + j, r)
        done_cp.append(out_cp(3 + j, pl.ds(3 * W + T * j, T), pl.ds(384, 512)))
        done_cp[-1].start()
    for cp in done_cp:
        cp.wait()


def _in_hbm(a):
    return pltpu.with_memory_space_constraint(a, pltpu.MemorySpace.HBM)


@jax.jit
def pallas_concat_heads__ssm_conv_s4__grouped_kv_mqa__prompt_kernel(
    A_u: jax.Array,
    A_A_re: jax.Array,
    A_A_im: jax.Array,
    A_B_re: jax.Array,
    A_B_im: jax.Array,
    A_C_re: jax.Array,
    A_C_im: jax.Array,
    A_log_dt: jax.Array,
    A_Dskip: jax.Array,
    B_x: jax.Array,
    B_wq: jax.Array,
    B_wk: jax.Array,
    B_wv: jax.Array,
    B_wo: jax.Array,
):
    hbm = pl.BlockSpec(memory_space=pltpu.MemorySpace.HBM)
    scratch = [
        pltpu.VMEM((D, L), BF16),
        pltpu.VMEM((6, D, N), BF16),
        pltpu.VMEM((D,), BF16),
        pltpu.VMEM((D,), BF16),
        pltpu.VMEM((NB, D, T), BF16),
        pltpu.VMEM((D, D), BF16),
        pltpu.VMEM((DH, D), BF16),
        pltpu.VMEM((DH, D), BF16),
        pltpu.VMEM((D, D), BF16),
        pltpu.VMEM((10, 64, 256), U32),
        pltpu.VMEM((2, 32, 128), U32),
        pltpu.VMEM((L, 2 * D), BF16),
        pltpu.VMEM((256, D), U32),
        pltpu.VMEM((D // 2, D), U32),
        pltpu.VMEM((NB, D, T), F32),
        pltpu.VMEM((L // 2, 128), U32),
        pltpu.VMEM((2, 16, L), U32),
        pltpu.VMEM((L, W), F32),
        pltpu.VMEM((NB, D, T), F32),
        pltpu.VMEM((2, 512, 128), F32),
        pltpu.VMEM((D, 128), F32),
        pltpu.VMEM((2, D, N), F32),
        pltpu.VMEM((2 * GA, 12, 72, 128), F32),
        pltpu.VMEM((2 * GA, 44, 8, 128), F32),
        pltpu.VMEM((D // 32, 32 * PST, 128), F32),
        pltpu.VMEM((NB, D // 2, 128), U32),
        pltpu.VMEM((2, 2, D, 128), F32),
        pltpu.VMEM((D // 8, 3 * NB, 8, 128), F32),
        pltpu.VMEM((D // 8, 3 * NB, 8, 128), F32),
        pltpu.VMEM((NB, 2, D, 128), F32),
        pltpu.VMEM((2, 4, T, 128), F32),
        pltpu.VMEM((8, 128), U32),
        pltpu.SemaphoreType.DMA((NB,)),
        pltpu.SemaphoreType.DMA((D // 32,)),
        pltpu.SemaphoreType.DMA((15,)),
        pltpu.SemaphoreType.DMA((7,)),
    ]
    return pl.pallas_call(
        _kernel,
        out_shape=jax.ShapeDtypeStruct((1, L, 2 * D), BF16),
        in_specs=[hbm] * 16,
        out_specs=hbm,
        scratch_shapes=scratch,
        compiler_params=pltpu.CompilerParams(vmem_limit_bytes=100 * 2**20),
    )(*map(_in_hbm, (A_u.transpose(0, 2, 1), A_A_re, A_A_im, A_B_re, A_B_im, A_C_re, A_C_im, A_log_dt, A_Dskip,
                     B_x.transpose(0, 2, 1), B_wq, B_wk.T, B_wv.T, B_wo, jnp.asarray(_FWD), jnp.asarray(_INV))))
```

```python
import ml_dtypes
import numpy as np

import jax
import jax.numpy as jnp
from jax import lax
import jax.experimental.pallas as pl
import jax.experimental.pallas.tpu as pltpu

L = 2048
D = 448
N = 256
H = 16
DH = 28
W = 512
CH = 128
NCH = L // CH
T = 128
NB = L // T
GA = 4
GC = 5
PW = 1
PST = 9
PEEL = 2
Z0, Z1, Z2 = 4, 7, 12
LAG_P, LAG_A, LAG_C = 2, 3, 1
CONV_STEP = 2
UP, NU = 4, 8
QP, NQ = 1, 54
OP, OL, NO = 15, 3, 14
KP_AT, KP_LAG = 18, 1
WO_AT = 12
LAST_AT = (14, 18, 22, 26)
F32 = jnp.float32
BF16 = jnp.bfloat16
U32 = jnp.uint32
NT_DIMS = (((1,), (1,)), ((), ()))

HI = (1, 2, 3, 4, 258, 260, 516, 772)
LO = tuple(4 * a for a in range(64)) + tuple(1028 + 8 * b for b in range(32))
POWER_PLAN = (
    ("x", 0, 1), ("z", 1, 1), ("x", 0, 2), ("x", 1, 2), ("x", 2, 2), ("z", 2, 2), ("z", 4, 4), ("z", 8, 4), ("z", 8, 8),
    ("z", 16, 4), ("z", 16, 12), ("z", 16, 8), ("z", 16, 16), ("z", 32, 8), ("z", 32, 16), ("z", 32, 24),
    ("z", 32, 32), ("z", 64, 32), ("z", 64, 64), ("z", 128, 32), ("z", 128, 96), ("z", 128, 64), ("z", 128, 128),
    ("x", 2, 256), ("x", 4, 256), ("z", 256, 256), ("x", 4, 512), ("x", 260, 512), ("z", 512, 512),
    ("z", 1024, 4), ("z", 1028, 64), ("z", 1028, 128), ("z", 1028, 192))
T_OF_BLOCK = (0, 1, 2, 3, 4, 5, 6, 7, 8, 9, 10, 11, 12, 5, 13, 7)
M_OF_BLOCK = (0, 1, 2, 3, 4, 5, 4, 5, 6, 7, 8, 7, 8, 7, 8, 7)


def _pack_np(a):
    bits = a.astype(np.float32).astype(ml_dtypes.bfloat16).view(np.uint16).astype(np.uint32)
    return bits[..., 0::2, :] | (bits[..., 1::2, :] << 16)


def _pack(a):
    return pltpu.bitcast(a.astype(BF16), jnp.uint32)


def _unpack(a):
    return pltpu.bitcast(a, BF16)


def _constants():
    f = np.arange(64)
    theta = np.pi * (2 * f + 1) / 256.0
    theta = np.concatenate([theta, -(np.pi * (2 * (127 - f) + 1) / 256.0)])

    def fwd(pos):
        ang = np.asarray(pos, np.float64)[:, None] * theta[None, :]
        return np.concatenate([np.cos(ang), -np.sin(ang)], axis=1)

    lane = np.arange(128)
    rows = [np.array([h + lo for lo in LO] + [-1] * 32) for h in HI]
    x01 = np.where(lane < 64, rows[0], np.roll(rows[1], 64))
    x23 = np.where(lane < 64, rows[2], np.roll(rows[3], 64))
    t2 = np.where(lane < 64, rows[4], np.roll(rows[5], 64))
    packed = [
        np.where((lane & 32) == 0, x01, np.roll(x23, 32)),
        np.where((lane & 32) != 0, x01, np.roll(x23, 96)),
        np.where(lane == 63, rows[3], t2), t2,
        np.where(lane == 63, rows[5], rows[6]), rows[6],
        np.where(lane == 63, rows[6], rows[7]), rows[7],
        np.where(lane == 63, rows[7], rows[3]), rows[3],
        np.where(lane == 95, rows[3], rows[5]), rows[5],
        np.where(lane == 95, rows[5], rows[6]),
        np.where(lane == 95, rows[6], rows[7]),
    ]
    lag_bf16 = np.arange(L + 1).astype(np.float32).astype(ml_dtypes.bfloat16).astype(np.int64)
    mats = {}
    for blk in range(NB):
        held = packed[T_OF_BLOCK[blk]]
        m = np.zeros((128, 256))
        for r in range(1, T + 1):
            (src,) = np.nonzero(held == lag_bf16[T * blk + r])
            m[src[0]] += fwd([r])[0]
        prev = mats.setdefault(M_OF_BLOCK[blk], m)
        assert np.array_equal(prev, m)
    fw = np.stack([mats[i] for i in range(9)] + [fwd(np.arange(T))])
    inv = []
    for par in range(2):
        ang = (2 * np.arange(64) + par)[:, None] * theta[None, :64]
        inv.append(np.concatenate([np.cos(ang), -np.sin(ang)], axis=1) / 128.0)
    return _pack_np(fw), _pack_np(np.stack(inv))


_FWD, _INV = _constants()


def _cmul(a, b):
    return a[0] * b[0] - a[1] * b[1], a[0] * b[1] + a[1] * b[0]


def _token(*values):
    tok = None
    for v in values:
        v = pltpu.bitcast(v, U32)
        for r in range(0, v.shape[0], 8):
            for c in range(0, v.shape[1], 128):
                tile = v[r:r + 8, c:c + 128]
                tok = tile if tok is None else tok | tile
    return tok


def chain(*gens):
    for gen in gens:
        yield from gen


def _kernel(u_hbm, are_hbm, aim_hbm, bre_hbm, bim_hbm, cre_hbm, cim_hbm, ldt_hbm, dsk_hbm,
            x_hbm, wq_hbm, wk_hbm, wv_hbm, wo_hbm, fw_hbm, inv_hbm,
            out_hbm,
            u_v, par_v, ldt_v, dsk_v, x_v, wq_v, wk_v, wv_v, wo_v, fw_v, inv_v, out_v,
            wt, wot, qt, kc, vtc, s_buf, ot, dtc, k0c, z1, pw, mul, kbuf, tbuf, hlast, gbuf, zero_ref, ubuf, ybuf, yst,
            x_sem, u_sem, in_sem, out_sem):
    def x_cp(i):
        tok = pl.ds(i * T if isinstance(i, int) else pl.multiple_of(i * T, T), T)
        return pltpu.make_async_copy(x_hbm.at[0, :, tok], x_v.at[i], x_sem.at[i])

    def u_cp(i):
        rows = pl.ds(i * 32 if isinstance(i, int) else pl.multiple_of(i * 32, 32), 32)
        return pltpu.make_async_copy(u_hbm.at[0, rows], u_v.at[rows], u_sem.at[i])

    pairs = [(r, par_v.at[i]) for i, r in enumerate((are_hbm, aim_hbm, bre_hbm, bim_hbm, cre_hbm, cim_hbm))]
    pairs += [(ldt_hbm, ldt_v), (dsk_hbm, dsk_v), (wq_hbm, wq_v), (wk_hbm, wk_v), (wv_hbm, wv_v),
              (fw_hbm.at[9], fw_v.at[9]), (fw_hbm.at[pl.ds(0, 9)], fw_v.at[pl.ds(0, 9)]), (wo_hbm, wo_v), (inv_hbm, inv_v)]
    cps = [pltpu.make_async_copy(src, dst, in_sem.at[i]) for i, (src, dst) in enumerate(pairs)]
    first_cp, weight_cp, second_cp, late_cp = [cps[6]] + cps[:2], cps[8:11], cps[2:6] + [cps[7], cps[11]], cps[12:]
    for cp in first_cp + weight_cp + [x_cp(i) for i in range(4)]:
        cp.start()

    def pad_rows(a, rows):
        return jnp.concatenate([a, jnp.zeros((rows - a.shape[0], a.shape[1]), a.dtype)], axis=0)

    def transpose_weight(w_ref, dst, panels=(0, 1, 2, 3)):
        for j in panels:
            wd = min(128, D - 128 * j)
            panel = w_ref[:, 128 * j:128 * j + wd].astype(F32)
            if wd < 128:
                panel = jnp.concatenate([panel, jnp.zeros((D, 128 - wd), F32)], axis=1)
            words = _pack(pad_rows(panel, 512).T[:wd, :D])
            dst[64 * j:64 * j + wd // 2, :] = words
        return words[:8, :128]

    def to_column(row):
        row = jnp.concatenate([row, jnp.zeros((1, 512 - D), F32)], axis=1)
        return jnp.broadcast_to(row, (128, 512)).T

    def tie(words, tokens):
        if not tokens:
            return words
        zero = zero_ref[:8]
        rows = [words[r:r + 8] for r in range(0, words.shape[0], 8)]
        for i, tok in enumerate(tokens):
            r = max((i + 1) * len(rows) // len(tokens) - 1, 0)
            first = rows[r][:, :128] | (tok & zero)
            rows[r] = first if words.shape[1] == 128 else jnp.concatenate([first, rows[r][:, 128:]], axis=1)
        return jnp.concatenate(rows, axis=0)

    def project_q(blk, tokens=()):
        qt[blk] = jnp.dot(_unpack(tie(wt[:D // 2, :], tokens)), x_v[blk], preferred_element_type=F32)

    def project_kv(i):
        tok = pl.ds(pl.multiple_of(i * W, W), W)
        x_t = jnp.concatenate([x_v[4 * i + j] for j in range(4)], axis=1)
        pr = jnp.dot(_unpack(wt[D // 2:, :]), x_t, preferred_element_type=F32)
        k_t, v_t = pr[:32], pr[32:]
        row32 = lax.broadcasted_iota(jnp.int32, (32, W), 0)
        k_both = pad_rows(jnp.concatenate([k_t, pltpu.roll(k_t, 4, 0)], axis=0), 128).T
        kc[pl.ds(pl.multiple_of(i * (W // 2), W // 2), W // 2), :] = _pack(k_both)
        for par in range(2):
            v_p = v_t if par == 0 else pltpu.roll(v_t, 4, 0)
            vtc[par, :, tok] = _pack(jnp.where(row32 == (DH if par == 0 else 0), 1.0, v_p))

    def q_window(pair, par):
        start = pl.multiple_of((pair % 8) * 56 + 24 * par, 8)
        q = jnp.concatenate([qt[4 * (pair // 8) + j, pl.ds(start, 32), :] for j in range(4)], axis=1)
        q = (q * np.float32(DH ** -0.5 * np.log2(np.e))).astype(BF16)
        zero = jnp.zeros((32, W), BF16)
        return jnp.concatenate([q, zero] if par == 0 else [zero, q], axis=0)

    def step(q_next, par_cur, mx_cur, fill, pending, pv_first=False):
        state = {}

        def scores(c, due):
            k_c = tie(kc[c * CH // 2:(c + 1) * CH // 2, :], due)
            s = jnp.dot(_unpack(k_c)[:, :64], q_next, preferred_element_type=F32)
            s_buf[c * CH:(c + 1) * CH, :] = s
            t = jnp.max(s.reshape(CH // 8, 8, W), axis=0)
            state["max"] = jnp.maximum(state["max"], t) if c else t

        def values(c, p, due):
            v_t = tie(vtc[par_cur, :, c * CH:(c + 1) * CH], due)
            o = jnp.dot(_unpack(v_t), p, preferred_element_type=F32)
            state["acc"] = state["acc"] + o if c else o

        if par_cur is not None:
            row_max = jnp.broadcast_to(jnp.max(mx_cur, axis=0, keepdims=True), (8, W))
        for c in range(NCH):
            due = pending.pop(0)
            if par_cur is None:
                scores(c, due)
            else:
                z = s_buf[c * CH:(c + 1) * CH, :].reshape(CH // 8, 8, W) - row_max[None]
                p = jnp.exp2(z).reshape(CH, W).astype(BF16)
                if q_next is None:
                    values(c, p, due)
                elif pv_first and c == NCH - 1:
                    values(c, p, [])
                    scores(c, due)
                else:
                    scores(c, due)
                    values(c, p, [])
            pending.append(fill(c))
        return state.get("max"), state.get("acc")

    def head_pair(pair, m, fill, lag=2, last=False):
        pending = [[]] * lag
        m, even = step(q_window(pair, 1), 0, m, fill, pending)
        m, odd = step(None if last else q_window(pair + 1, 0), 1, m, lambda c: fill(NCH + c), pending,
                      True)
        even = even * (1.0 / even[DH:DH + 1])
        odd = odd * (1.0 / odd[0:1])
        mid = jnp.where(lax.broadcasted_iota(jnp.int32, (8, W), 0) < 4, even[24:32], odd[0:8])
        rows = pl.ds(pl.multiple_of((pair % 8) * 56, 8), 56)
        o_t = jnp.concatenate([even[:24], mid, odd[8:]], axis=0)
        for j in range(4):
            ot[4 * (pair // 8) + j, rows, :] = o_t[:, j * T:(j + 1) * T]
        return m

    def out_features(blk, lo, hi, tokens=()):
        return jnp.dot(_unpack(tie(wot[:, lo:hi], tokens)), ot[blk, lo:hi, :].astype(BF16), preferred_element_type=F32)

    def put_out(blk, r):
        r = jnp.concatenate([jnp.zeros((64, T), F32), r], axis=0).T.astype(BF16)
        rows = pl.ds(blk * T if isinstance(blk, int) else pl.multiple_of(blk * T, T), T)
        out_v[rows, D:512] = r[:, 64:128]
        out_v[rows, 512:] = r[:, 128:]
        return _token(r)

    def discretize(g):
        rows = pl.ds(g * 8 if isinstance(g, int) else pl.multiple_of(g * 8, 8), 8)
        dt = dtc[0, rows, :]
        for lanes in (slice(0, 128), slice(128, 256)):
            mag = jnp.exp(dt * par_v[0, rows, lanes].astype(F32))
            ang = dt * par_v[1, rows, lanes].astype(F32)
            re, im = mag * jnp.cos(ang), mag * jnp.sin(ang)
            z1[0, rows, lanes], z1[1, rows, lanes] = re, im
            yield _token(re, im)

    def modes(first, count):
        return chain(*(discretize(first + j) for j in range(count)))

    def powers(g, slot):
        n = 8 * PW
        rows = pl.ds(pl.multiple_of(g * 8, n), n)
        dt = dtc[0, rows, :]
        dt = jnp.concatenate([dt, dt], axis=1)
        b_re, b_im, c_re, c_im = (par_v[i, rows, :].astype(F32) for i in range(2, 6))
        w = _cmul((c_re, c_im), (dt * b_re, dt * b_im))
        k0c[rows, :] = jnp.sum(w[0], axis=1, keepdims=True) + dtc[1, rows, :]
        yield _token(w[1])
        z = {0: (jnp.ones((n, N), F32), jnp.zeros((n, N), F32)), 1: (z1[0, rows, :], z1[1, rows, :])}

        def tiles(v):
            return [(j, part, half, v[part][8 * j:8 * j + 8, 128 * half:128 * (half + 1)])
                    for j in range(PW) for part in range(2) for half in range(2)]

        def put_strided(i, s, v):
            for j, part, half, tile in tiles(v):
                pw[slot + j, 4 * i + 2 * part + half, pl.ds(s, 8, stride=PST), :] = tile

        def put(p):
            if p in LO[8::8]:
                for j, part, half, tile in tiles(z[p]):
                    mul[slot + j, 4 * LO[8::8].index(p) + 2 * half + part] = tile
            if p < 32 and p % 4 == 0:
                put_strided(0, p // 4, z[p])
            if p < 64 and p % 8 == 0:
                put_strided(1, p // 8, z[p])

        put(0)
        x = {0: w}
        for kind, p, q in POWER_PLAN:
            if kind == "x":
                x[p + q] = _cmul(x[p], z[q])
                put_strided(2, HI.index(p + q), (x[p + q][0], -x[p + q][1]))
                yield _token(x[p + q][1])
                continue
            re, im = z[p]
            z[p + q] = (re * re - im * im, 2.0 * (re * im)) if p == q else _cmul(z[p], z[q])
            put(p + q)
            yield _token(z[p + q][0])

    def kernel_channel(g, j, slot, c):
        rows = slice(PST * c, PST * c + 8)
        taps = None
        for half in range(2):
            step4, step8, lhs = ([pw[slot, 4 * i + 2 * part + half, rows, :] for part in range(2)] for i in range(3))
            grp = [step4]
            for i in range(11):
                m_i = [jnp.broadcast_to(mul[slot, 4 * i + 2 * half + part, c:c + 1, :], (8, 128)) for part in range(2)]
                grp.append(_cmul(step4 if i < 7 else step8, m_i))
            rhs = jnp.concatenate([jnp.concatenate([v[part] for v in grp], axis=0) for part in range(2)], axis=1)
            rhs, lhs = pad_rows(rhs, 128), jnp.concatenate(lhs, axis=1)
            t = lax.dot_general(lhs, rhs, NT_DIMS, preferred_element_type=F32)
            taps = t if taps is None else taps + t
        kbuf[g // 4, PST * (8 * j + c):PST * (8 * j + c) + 8, :] = taps

    def pack_taps(i):
        lane = lax.broadcasted_iota(jnp.int32, (32, 128), 1)
        r = [kbuf[i, pl.ds(j, 32, stride=PST), :] for j in range(8)]
        x01 = jnp.where(lane < 64, r[0], pltpu.roll(r[1], 64, 1))
        x23 = jnp.where(lane < 64, r[2], pltpu.roll(r[3], 64, 1))
        t2 = jnp.where(lane < 64, r[4], pltpu.roll(r[5], 64, 1))
        packed = [
            jnp.where((lane & 32) == 0, x01, pltpu.roll(x23, 32, 1)),
            jnp.where((lane & 32) != 0, x01, pltpu.roll(x23, 96, 1)),
            jnp.where(lane == 63, r[3], t2), t2,
            jnp.where(lane == 63, r[5], r[6]), r[6],
            jnp.where(lane == 63, r[6], r[7]), r[7],
            jnp.where(lane == 63, r[7], r[3]), r[3],
            jnp.where(lane == 95, r[3], r[5]), r[5],
            jnp.where(lane == 95, r[5], r[6]),
            jnp.where(lane == 95, r[6], r[7]),
        ]
        for blk in range(NB):
            tbuf[blk, pl.ds(pl.multiple_of(i * 16, 16), 16), :] = _pack(packed[T_OF_BLOCK[blk]])
        return _token(packed[0], packed[1], packed[2])

    def taps_dft(blk, slot):
        mat = jnp.where(blk < 6, blk, jnp.where(blk < 8, blk - 2, jnp.where(blk == 8, 6, 8 - blk % 2)))
        h = jnp.dot(_unpack(tbuf[blk]), _unpack(fw_v[mat]), preferred_element_type=F32)
        h_re, h_im = h[:, :128], h[:, 128:]
        g_re, g_im = h_re + hlast[1 - slot, 0], h_im + hlast[1 - slot, 1]
        even = (lax.broadcasted_iota(jnp.int32, (D, 128), 1) & 1) == 0
        hlast[slot, 0] = jnp.where(even, -1.0, 1.0) * h_im
        hlast[slot, 1] = jnp.where(even, 1.0, -1.0) * h_re
        g_dif, g_sum = g_im - g_re, g_re + g_im
        for t, v in enumerate((g_re, g_dif, g_sum)):
            gbuf[:, 3 * blk + t] = v.reshape(D // 8, 8, 128)

    def input_dft(g, b0, nb, tokens):
        rows = pl.ds(pl.multiple_of(g * 8, 8 * GA), 8 * GA)
        u_t = jnp.concatenate([u_v[rows, b * T:(b + 1) * T] for b in range(b0, b0 + nb)], axis=0)
        r = jnp.dot(_unpack(tie(_pack(u_t), tokens)), _unpack(fw_v[9]), preferred_element_type=F32)
        for b in range(nb):
            u_re, u_im = r[8 * GA * b:8 * GA * (b + 1), :128], r[8 * GA * b:8 * GA * (b + 1), 128:]
            for t, v in enumerate((u_re + u_im, u_re, u_im)):
                ubuf[pl.ds(g, GA), 3 * (b0 + b) + t] = v.reshape(GA, 8, 128)

    def block_conv(g, k):
        rows = pl.ds(pl.multiple_of(g * 8, 8), 8)
        low = lax.broadcasted_iota(jnp.int32, (8, 128), 1) < 64
        acc, loaded = {}, {}

        def g_at(d, t):
            if (d, t) not in loaded:
                loaded[d, t] = gbuf[g, 3 * d + t]
            return loaded[d, t]

        for j in range(2 * k + 2):
            if j and j % CONV_STEP == 0:
                yield _token(acc[2 * k + 1][2])
            u_j = [ubuf[g, 3 * j + t] for t in range(3)]
            for i in range(max(j, 2 * k), 2 * k + 2):
                prod = [g_at(i - j, t) * u_j[t] for t in range(3)]
                acc[i] = [a + b for a, b in zip(acc[i], prod)] if i in acc else prod
        done = []
        for i, (k1, k2, k3) in acc.items():
            y_re, y_im = k1 - k3, k1 + k2
            swapped = pltpu.roll(jnp.where(low, y_im, y_re), 64, 1)
            first = jnp.where(low, y_re, swapped)
            second = jnp.where(low, swapped, y_im)
            done += [first + second, first - second]
            ybuf[i, 0, rows, :], ybuf[i, 1, rows, :] = done[-2:]
        yield _token(*done)

    def inverse_dft(blk, slot):
        for par in range(2):
            y = lax.dot_general(_unpack(inv_v[par]), pad_rows(ybuf[blk, par], 512).astype(BF16), NT_DIMS,
                                preferred_element_type=F32)
            for j in range(4):
                yst[slot, j, pl.ds(par, 64, stride=2), :] = y[:, 128 * j:128 * (j + 1)]
        rows = pl.ds(blk * T, T)
        for j in range(4):
            wd = min(128, D - 128 * j)
            out_v[rows, 128 * j:128 * j + wd] = yst[slot, j, :T, :].astype(BF16)[:, :wd]

    zero_ref[...] = jnp.zeros(zero_ref.shape, U32)
    for cp in first_cp:
        cp.wait()
    dtc[0] = to_column(jnp.exp(ldt_v[...].astype(F32).reshape(1, D)).astype(BF16).astype(F32))
    for cp in [x_cp(i) for i in range(4, NB)]:
        cp.start()

    @pl.loop(0, 4)
    def _(i):
        list(modes(Z0 * i, Z0))

    kbuf[0] = jnp.zeros(kbuf.shape[1:], F32)
    for cp in weight_cp:
        cp.wait()
    for i, w_ref in enumerate((wk_v, wv_v)):
        wt[D // 2 + 16 * i:D // 2 + 16 * (i + 1), :] = _pack(pad_rows(w_ref[...].astype(F32), 32))
    transpose_weight(wq_v, wt)

    def prologue(i, carry):
        for j in range(4):
            x_cp(4 * i + j).wait()
        project_kv(i)
        project_q(i, list(modes(4 * Z0 + Z1 * i, Z1)))
        return carry

    for cp in second_cp:
        cp.start()
    lax.fori_loop(0, 4, prologue, 0)
    early = list(modes(4 * (Z0 + Z1), Z2))
    m, _ = step(q_window(0, 0), None, None,
                lambda c: early[c * 2 * Z2 // (NCH - 2):(c + 1) * 2 * Z2 // (NCH - 2)], [[], []])
    for cp in second_cp:
        cp.wait()
    for cp in [u_cp(i) for i in range(D // 32)] + late_cp:
        cp.start()
    dtc[1] = to_column(dsk_v[...].astype(F32).reshape(1, D))

    def spread(streams, lag=2):
        span = 2 * NCH - lag

        def fill(c):
            out = []
            for gen, count in streams:
                count = span if count is None else count
                if c < span:
                    out += [next(gen) for _ in range((c + 1) * count // span - c * count // span)]
                if c == span - 1 and count != span:
                    assert next(gen, fill) is fill
            return [t for t in out if t is not None]
        return fill

    def once(job, at, lag=0):
        def gen():
            yield from [None] * at
            done = job()
            yield from [None] * lag + [done] + [None] * (2 * NCH)
        return gen(), None

    last_group = D // 8 - 1
    n_a = -(-(D // 8) // GA)
    n_c = -(-(D // 8) // GC)

    def phase_p(it, m):
        ahead = chain(*(powers(2 * it + j, 2 * it + j) for j in range(2)))
        n = (D // 8 - 4 * (Z0 + Z1) - Z2) // 2
        streams = [(ahead, 2 * (1 + len(POWER_PLAN))), (modes(D // 8 - n * (2 - it), n), 2 * n)]
        return head_pair(it, m, spread(streams, LAG_P), LAG_P)

    m = lax.fori_loop(0, 2, phase_p, m)

    def phase_a(it, m, query=True, more=True):
        u_cp(it).wait()
        cur, nxt = (it % 2) * GA, (1 - it % 2) * GA
        taps = (kernel_channel(GA * it + j, j, cur + j, c) for j in range(GA) for c in range(8))
        ahead = chain(*(powers(jnp.minimum(GA * (it + 1) + j, D // 8 - PW), nxt + j) for j in range(0, GA, PW)))

        def take(n):
            return [next(ahead) for _ in range(n if more else 0)]

        n_tok = (1 + len(POWER_PLAN)) * GA // PW - UP * NU
        streams = [once(lambda: pack_taps(jnp.maximum(it - 1, 0)), KP_AT, KP_LAG)]
        if query:
            streams.append(once(lambda: project_q(jnp.minimum(4 + it, NB - 1), take(NQ)), QP))
        else:
            streams.append(once(lambda: transpose_weight(wo_v, wot, (0, 1) if more else (2, 3)), WO_AT, 6))
        streams += [(taps, 8 * GA), ((input_dft(GA * it, b, NB // UP, take(NU)) for b in range(0, NB, NB // UP)), UP)]
        if more:
            streams.append((ahead, n_tok - (NQ if query else 0)))
        m = head_pair(2 + it, m, spread(streams, LAG_A), LAG_A)
        return m

    m = lax.fori_loop(0, n_a - PEEL, phase_a, m)
    for cp in late_cp:
        cp.wait()
    for it in range(n_a - PEEL, n_a):
        m = phase_a(jnp.int32(it), m, query=False, more=it + 1 < n_a)
    pack_taps(n_a - 1)
    hlast[1, 0] = k0c[...]
    hlast[1, 1] = jnp.zeros((D, 128), F32)

    def phase_b(it, m):
        return head_pair(16 + it, m, spread([((taps_dft(8 * it + j, j % 2) for j in range(8)), 8)]))

    m = lax.fori_loop(0, 2, phase_b, m)

    def phase_c(it, m):
        convs = chain(*(block_conv(jnp.minimum(GC * it + j, last_group), k)
                        for j in range(GC) for k in range(8)))
        count = GC * sum(1 + (2 * k + 1) // CONV_STEP for k in range(8))
        proj = once(lambda: put_out(it, out_features(it, 0, D, [next(convs) for _ in range(NO)])), OP, OL)
        return head_pair(18 + it, m, spread([proj, (convs, count - NO)], LAG_C), LAG_C)

    m = lax.fori_loop(0, n_c, phase_c, m)

    def out_cp(i, rows, cols):
        return pltpu.make_async_copy(out_v.at[rows, cols], out_hbm.at[0, rows, cols], out_sem.at[i])

    done_cp = [out_cp(0, pl.ds(0, 3 * W), pl.ds(512, 384))]
    done_cp[0].start()
    m = head_pair(30, m, spread([((inverse_dft(blk, blk % 2) for blk in range(NB)), NB)]))
    done_cp += [out_cp(1, pl.ds(0, 3 * W), pl.ds(0, 512)), out_cp(2, pl.ds(3 * W, W), pl.ds(0, 384))]
    for cp in done_cp[1:]:
        cp.start()

    def fill_last(c):
        if c in LAST_AT:
            j = LAST_AT.index(c)
            qt[j] = out_features(12 + j, 0, 384)
        return []

    head_pair(31, m, fill_last, last=True)
    tails = [qt[j] + out_features(12 + j, 384, D) for j in range(W // T)]
    for j, r in enumerate(tails):
        put_out(12 + j, r)
        done_cp.append(out_cp(3 + j, pl.ds(3 * W + T * j, T), pl.ds(384, 512)))
        done_cp[-1].start()
    for cp in done_cp:
        cp.wait()


@jax.jit
def pallas_concat_heads__ssm_conv_s4__grouped_kv_mqa__prompt_kernel(
    A_u: jax.Array,
    A_A_re: jax.Array,
    A_A_im: jax.Array,
    A_B_re: jax.Array,
    A_B_im: jax.Array,
    A_C_re: jax.Array,
    A_C_im: jax.Array,
    A_log_dt: jax.Array,
    A_Dskip: jax.Array,
    B_x: jax.Array,
    B_wq: jax.Array,
    B_wk: jax.Array,
    B_wv: jax.Array,
    B_wo: jax.Array,
):
    hbm = pl.BlockSpec(memory_space=pltpu.MemorySpace.HBM)
    scratch = [
        pltpu.VMEM((D, L), BF16),
        pltpu.VMEM((6, D, N), BF16),
        pltpu.VMEM((D,), BF16),
        pltpu.VMEM((D,), BF16),
        pltpu.VMEM((NB, D, T), BF16),
        pltpu.VMEM((D, D), BF16),
        pltpu.VMEM((DH, D), BF16),
        pltpu.VMEM((DH, D), BF16),
        pltpu.VMEM((D, D), BF16),
        pltpu.VMEM((10, 64, 256), U32),
        pltpu.VMEM((2, 32, 128), U32),
        pltpu.VMEM((L, 2 * D), BF16),
        pltpu.VMEM((256, D), U32),
        pltpu.VMEM((D // 2, D), U32),
        pltpu.VMEM((NB, D, T), F32),
        pltpu.VMEM((L // 2, 128), U32),
        pltpu.VMEM((2, 16, L), U32),
        pltpu.VMEM((L, W), F32),
        pltpu.VMEM((NB, D, T), F32),
        pltpu.VMEM((2, 512, 128), F32),
        pltpu.VMEM((D, 128), F32),
        pltpu.VMEM((2, D, N), F32),
        pltpu.VMEM((2 * GA, 12, 88, 128), F32),
        pltpu.VMEM((2 * GA, 44, 8, 128), F32),
        pltpu.VMEM((D // 32, 304, 128), F32),
        pltpu.VMEM((NB, D // 2, 128), U32),
        pltpu.VMEM((2, 2, D, 128), F32),
        pltpu.VMEM((D // 8, 3 * NB, 8, 128), F32),
        pltpu.VMEM((32, 128), U32),
        pltpu.VMEM((D // 8, 3 * NB, 8, 128), F32),
        pltpu.VMEM((NB, 2, D, 128), F32),
        pltpu.VMEM((2, 4, T + 8, 128), F32),
        pltpu.SemaphoreType.DMA((NB,)),
        pltpu.SemaphoreType.DMA((D // 32,)),
        pltpu.SemaphoreType.DMA((15,)),
        pltpu.SemaphoreType.DMA((7,)),
    ]
    return pl.pallas_call(
        _kernel,
        out_shape=jax.ShapeDtypeStruct((1, L, 2 * D), BF16),
        in_specs=[hbm] * 16,
        out_specs=hbm,
        scratch_shapes=scratch,
        compiler_params=pltpu.CompilerParams(vmem_limit_bytes=100 * 2**20),
    )(A_u.transpose(0, 2, 1), A_A_re, A_A_im, A_B_re, A_B_im, A_C_re, A_C_im, A_log_dt, A_Dskip,
      B_x.transpose(0, 2, 1), B_wq, B_wk.T, B_wv.T, B_wo, _FWD, _INV)
```

```python
import ml_dtypes
import numpy as np

import jax
import jax.numpy as jnp
from jax import lax
import jax.experimental.pallas as pl
import jax.experimental.pallas.tpu as pltpu

L = 2048
D = 448
N = 256
H = 16
DH = 28
W = 512
CH = 128
NCH = L // CH
T = 128
NB = L // T
GA = 4
GC = 5
PW = 1
PST = 9
PEEL = 2
Z0, Z1, Z2 = 4, 7, 12
LAG_P, LAG_A, LAG_C = 2, 3, 1
CONV_STEP = 2
UP, NU = 4, 8
QP, NQ = 1, 54
OP, OL, NO = 15, 3, 14
KP_AT, KP_LAG = 18, 1
WO_AT = 12
YS = 4
LAST_AT = (14, 18, 22, 26)
F32 = jnp.float32
BF16 = jnp.bfloat16
U32 = jnp.uint32
NT_DIMS = (((1,), (1,)), ((), ()))

HI = (1, 2, 3, 4, 258, 260, 516, 772)
LO = tuple(4 * a for a in range(64)) + tuple(1028 + 8 * b for b in range(32))
POWER_PLAN = (
    ("x", 0, 1), ("z", 1, 1), ("x", 0, 2), ("x", 1, 2), ("x", 2, 2), ("z", 2, 2), ("z", 4, 4), ("z", 8, 4), ("z", 8, 8),
    ("z", 16, 4), ("z", 16, 12), ("z", 16, 8), ("z", 16, 16), ("z", 32, 8), ("z", 32, 16), ("z", 32, 24),
    ("z", 32, 32), ("z", 64, 32), ("z", 64, 64), ("z", 128, 32), ("z", 128, 96), ("z", 128, 64), ("z", 128, 128),
    ("x", 2, 256), ("x", 4, 256), ("z", 256, 256), ("x", 4, 512), ("x", 260, 512), ("z", 512, 512),
    ("z", 1024, 4), ("z", 1028, 64), ("z", 1028, 128), ("z", 1028, 192))
T_OF_BLOCK = (0, 1, 2, 3, 4, 5, 6, 7, 8, 9, 10, 11, 12, 5, 13, 7)
M_OF_BLOCK = (0, 1, 2, 3, 4, 5, 4, 5, 6, 7, 8, 7, 8, 7, 8, 7)


def _pack_np(a):
    bits = a.astype(np.float32).astype(ml_dtypes.bfloat16).view(np.uint16).astype(np.uint32)
    return bits[..., 0::2, :] | (bits[..., 1::2, :] << 16)


def _pack(a):
    return pltpu.bitcast(a.astype(BF16), jnp.uint32)


def _unpack(a):
    return pltpu.bitcast(a, BF16)


def _constants():
    f = np.arange(64)
    theta = np.pi * (2 * f + 1) / 256.0
    theta = np.concatenate([theta, -(np.pi * (2 * (127 - f) + 1) / 256.0)])

    def fwd(pos):
        ang = np.asarray(pos, np.float64)[:, None] * theta[None, :]
        return np.concatenate([np.cos(ang), -np.sin(ang)], axis=1)

    lane = np.arange(128)
    rows = [np.array([h + lo for lo in LO] + [-1] * 32) for h in HI]
    x01 = np.where(lane < 64, rows[0], np.roll(rows[1], 64))
    x23 = np.where(lane < 64, rows[2], np.roll(rows[3], 64))
    t2 = np.where(lane < 64, rows[4], np.roll(rows[5], 64))
    packed = [
        np.where((lane & 32) == 0, x01, np.roll(x23, 32)),
        np.where((lane & 32) != 0, x01, np.roll(x23, 96)),
        np.where(lane == 63, rows[3], t2), t2,
        np.where(lane == 63, rows[5], rows[6]), rows[6],
        np.where(lane == 63, rows[6], rows[7]), rows[7],
        np.where(lane == 63, rows[7], rows[3]), rows[3],
        np.where(lane == 95, rows[3], rows[5]), rows[5],
        np.where(lane == 95, rows[5], rows[6]),
        np.where(lane == 95, rows[6], rows[7]),
    ]
    lag_bf16 = np.arange(L + 1).astype(np.float32).astype(ml_dtypes.bfloat16).astype(np.int64)
    mats = {}
    for blk in range(NB):
        held = packed[T_OF_BLOCK[blk]]
        m = np.zeros((128, 256))
        for r in range(1, T + 1):
            (src,) = np.nonzero(held == lag_bf16[T * blk + r])
            m[src[0]] += fwd([r])[0]
        prev = mats.setdefault(M_OF_BLOCK[blk], m)
        assert np.array_equal(prev, m)
    fw = np.stack([mats[i] for i in range(9)] + [fwd(np.arange(T))])
    inv = []
    for par in range(2):
        ang = (2 * np.arange(64) + par)[:, None] * theta[None, :64]
        inv.append(np.concatenate([np.cos(ang), -np.sin(ang)], axis=1) / 128.0)
    return _pack_np(fw), _pack_np(np.stack(inv))


_FWD, _INV = _constants()


def _cmul(a, b):
    return a[0] * b[0] - a[1] * b[1], a[0] * b[1] + a[1] * b[0]


def _token(*values):
    tok = None
    for v in values:
        v = pltpu.bitcast(v, U32)
        for r in range(0, v.shape[0], 8):
            for c in range(0, v.shape[1], 128):
                tile = v[r:r + 8, c:c + 128]
                tok = tile if tok is None else tok | tile
    return tok


def chain(*gens):
    for gen in gens:
        yield from gen


def _kernel(u_hbm, are_hbm, aim_hbm, bre_hbm, bim_hbm, cre_hbm, cim_hbm, ldt_hbm, dsk_hbm,
            x_hbm, wq_hbm, wk_hbm, wv_hbm, wo_hbm, fw_hbm, inv_hbm,
            out_hbm,
            u_v, par_v, ldt_v, dsk_v, x_v, wq_v, wk_v, wv_v, wo_v, fw_v, inv_v, out_v,
            wt, wot, qt, kc, vtc, s_buf, ot, dtc, k0c, z1, pw, mul, kbuf, tbuf, hlast, gbuf, zero_ref, ubuf, ybuf, yst,
            x_sem, u_sem, in_sem, out_sem):
    def x_cp(i):
        tok = pl.ds(i * T if isinstance(i, int) else pl.multiple_of(i * T, T), T)
        return pltpu.make_async_copy(x_hbm.at[0, :, tok], x_v.at[i], x_sem.at[i])

    def u_cp(i):
        rows = pl.ds(i * 32 if isinstance(i, int) else pl.multiple_of(i * 32, 32), 32)
        return pltpu.make_async_copy(u_hbm.at[0, rows], u_v.at[rows], u_sem.at[i])

    pairs = [(r, par_v.at[i]) for i, r in enumerate((are_hbm, aim_hbm, bre_hbm, bim_hbm, cre_hbm, cim_hbm))]
    pairs += [(ldt_hbm, ldt_v), (dsk_hbm, dsk_v), (wq_hbm, wq_v), (wk_hbm, wk_v), (wv_hbm, wv_v),
              (fw_hbm.at[9], fw_v.at[9]), (fw_hbm.at[pl.ds(0, 9)], fw_v.at[pl.ds(0, 9)]), (wo_hbm, wo_v), (inv_hbm, inv_v)]
    cps = [pltpu.make_async_copy(src, dst, in_sem.at[i]) for i, (src, dst) in enumerate(pairs)]
    first_cp, weight_cp, second_cp, late_cp = [cps[6]] + cps[:2], cps[8:11], cps[2:6] + [cps[7], cps[11]], cps[12:]
    for cp in first_cp + weight_cp + [x_cp(i) for i in range(4)]:
        cp.start()

    def pad_rows(a, rows):
        return jnp.concatenate([a, jnp.zeros((rows - a.shape[0], a.shape[1]), a.dtype)], axis=0)

    def transpose_weight(w_ref, dst, panels=(0, 1, 2, 3)):
        for j in panels:
            wd = min(128, D - 128 * j)
            panel = w_ref[:, 128 * j:128 * j + wd].astype(F32)
            if wd < 128:
                panel = jnp.concatenate([panel, jnp.zeros((D, 128 - wd), F32)], axis=1)
            words = _pack(pad_rows(panel, 512).T[:wd, :D])
            dst[64 * j:64 * j + wd // 2, :] = words
        return words[:8, :128]

    def to_column(row):
        row = jnp.concatenate([row, jnp.zeros((1, 512 - D), F32)], axis=1)
        return jnp.broadcast_to(row, (128, 512)).T

    def tie(words, tokens):
        if not tokens:
            return words
        zero = zero_ref[:8]
        rows = [words[r:r + 8] for r in range(0, words.shape[0], 8)]
        for i, tok in enumerate(tokens):
            r = max((i + 1) * len(rows) // len(tokens) - 1, 0)
            first = rows[r][:, :128] | (tok & zero)
            rows[r] = first if words.shape[1] == 128 else jnp.concatenate([first, rows[r][:, 128:]], axis=1)
        return jnp.concatenate(rows, axis=0)

    def project_q(blk, tokens=()):
        qt[blk] = jnp.dot(_unpack(tie(wt[:D // 2, :], tokens)), x_v[blk], preferred_element_type=F32)

    def project_kv(i):
        tok = pl.ds(pl.multiple_of(i * W, W), W)
        x_t = jnp.concatenate([x_v[4 * i + j] for j in range(4)], axis=1)
        pr = jnp.dot(_unpack(wt[D // 2:, :]), x_t, preferred_element_type=F32)
        k_t, v_t = pr[:32], pr[32:]
        row32 = lax.broadcasted_iota(jnp.int32, (32, W), 0)
        k_both = pad_rows(jnp.concatenate([k_t, pltpu.roll(k_t, 4, 0)], axis=0), 128).T
        kc[pl.ds(pl.multiple_of(i * (W // 2), W // 2), W // 2), :] = _pack(k_both)
        for par in range(2):
            v_p = v_t if par == 0 else pltpu.roll(v_t, 4, 0)
            vtc[par, :, tok] = _pack(jnp.where(row32 == (DH if par == 0 else 0), 1.0, v_p))

    def q_window(pair, par):
        start = pl.multiple_of((pair % 8) * 56 + 24 * par, 8)
        q = jnp.concatenate([qt[4 * (pair // 8) + j, pl.ds(start, 32), :] for j in range(4)], axis=1)
        q = (q * np.float32(DH ** -0.5 * np.log2(np.e))).astype(BF16)
        zero = jnp.zeros((32, W), BF16)
        return jnp.concatenate([q, zero] if par == 0 else [zero, q], axis=0)

    def step(q_next, par_cur, mx_cur, fill, pending, pv_first=False):
        state = {}

        def scores(c, due):
            k_c = tie(kc[c * CH // 2:(c + 1) * CH // 2, :], due)
            s = jnp.dot(_unpack(k_c)[:, :64], q_next, preferred_element_type=F32)
            s_buf[c * CH:(c + 1) * CH, :] = s
            t = jnp.max(s.reshape(CH // 8, 8, W), axis=0)
            state["max"] = jnp.maximum(state["max"], t) if c else t

        def values(c, p, due):
            v_t = tie(vtc[par_cur, :, c * CH:(c + 1) * CH], due)
            o = jnp.dot(_unpack(v_t), p, preferred_element_type=F32)
            state["acc"] = state["acc"] + o if c else o

        if par_cur is not None:
            row_max = jnp.broadcast_to(jnp.max(mx_cur, axis=0, keepdims=True), (8, W))
        for c in range(NCH):
            due = pending.pop(0)
            if par_cur is None:
                scores(c, due)
            else:
                z = s_buf[c * CH:(c + 1) * CH, :].reshape(CH // 8, 8, W) - row_max[None]
                p = jnp.exp2(z).reshape(CH, W).astype(BF16)
                if q_next is None:
                    values(c, p, due)
                elif pv_first and c == NCH - 1:
                    values(c, p, [])
                    scores(c, due)
                else:
                    scores(c, due)
                    values(c, p, [])
            pending.append(fill(c))
        return state.get("max"), state.get("acc")

    def head_pair(pair, m, fill, lag=2, last=False):
        pending = [[]] * lag
        m, even = step(q_window(pair, 1), 0, m, fill, pending)
        m, odd = step(None if last else q_window(pair + 1, 0), 1, m, lambda c: fill(NCH + c), pending,
                      True)
        even = even * (1.0 / even[DH:DH + 1])
        odd = odd * (1.0 / odd[0:1])
        mid = jnp.where(lax.broadcasted_iota(jnp.int32, (8, W), 0) < 4, even[24:32], odd[0:8])
        rows = pl.ds(pl.multiple_of((pair % 8) * 56, 8), 56)
        o_t = jnp.concatenate([even[:24], mid, odd[8:]], axis=0)
        for j in range(4):
            ot[4 * (pair // 8) + j, rows, :] = o_t[:, j * T:(j + 1) * T]
        return m

    def out_features(blk, lo, hi, tokens=()):
        return jnp.dot(_unpack(tie(wot[:, lo:hi], tokens)), ot[blk, lo:hi, :].astype(BF16), preferred_element_type=F32)

    def put_out(blk, r):
        r = jnp.concatenate([jnp.zeros((64, T), F32), r], axis=0).T.astype(BF16)
        rows = pl.ds(blk * T if isinstance(blk, int) else pl.multiple_of(blk * T, T), T)
        out_v[rows, D:512] = r[:, 64:128]
        out_v[rows, 512:] = r[:, 128:]
        return _token(r)

    def discretize(g):
        rows = pl.ds(g * 8 if isinstance(g, int) else pl.multiple_of(g * 8, 8), 8)
        dt = dtc[0, rows, :]
        for lanes in (slice(0, 128), slice(128, 256)):
            mag = jnp.exp(dt * par_v[0, rows, lanes].astype(F32))
            ang = dt * par_v[1, rows, lanes].astype(F32)
            re, im = mag * jnp.cos(ang), mag * jnp.sin(ang)
            z1[0, rows, lanes], z1[1, rows, lanes] = re, im
            yield _token(re, im)

    def modes(first, count):
        return chain(*(discretize(first + j) for j in range(count)))

    def powers(g, slot):
        n = 8 * PW
        rows = pl.ds(pl.multiple_of(g * 8, n), n)
        dt = dtc[0, rows, :]
        dt = jnp.concatenate([dt, dt], axis=1)
        b_re, b_im, c_re, c_im = (par_v[i, rows, :].astype(F32) for i in range(2, 6))
        w = _cmul((c_re, c_im), (dt * b_re, dt * b_im))
        k0c[rows, :] = jnp.sum(w[0], axis=1, keepdims=True) + dtc[1, rows, :]
        yield _token(w[1])
        z = {0: (jnp.ones((n, N), F32), jnp.zeros((n, N), F32)), 1: (z1[0, rows, :], z1[1, rows, :])}

        def tiles(v):
            return [(j, part, half, v[part][8 * j:8 * j + 8, 128 * half:128 * (half + 1)])
                    for j in range(PW) for part in range(2) for half in range(2)]

        def put_strided(i, s, v):
            for j, part, half, tile in tiles(v):
                pw[slot + j, 4 * i + 2 * part + half, pl.ds(s, 8, stride=PST), :] = tile

        def put(p):
            if p in LO[8::8]:
                for j, part, half, tile in tiles(z[p]):
                    mul[slot + j, 4 * LO[8::8].index(p) + 2 * half + part] = tile
            if p < 32 and p % 4 == 0:
                put_strided(0, p // 4, z[p])
            if p < 64 and p % 8 == 0:
                put_strided(1, p // 8, z[p])

        put(0)
        x = {0: w}
        for kind, p, q in POWER_PLAN:
            if kind == "x":
                x[p + q] = _cmul(x[p], z[q])
                put_strided(2, HI.index(p + q), (x[p + q][0], -x[p + q][1]))
                yield _token(x[p + q][1])
                continue
            re, im = z[p]
            z[p + q] = (re * re - im * im, 2.0 * (re * im)) if p == q else _cmul(z[p], z[q])
            put(p + q)
            yield _token(z[p + q][0])

    def kernel_channel(g, j, slot, c):
        rows = slice(PST * c, PST * c + 8)
        taps = None
        for half in range(2):
            step4, step8, lhs = ([pw[slot, 4 * i + 2 * part + half, rows, :] for part in range(2)] for i in range(3))
            grp = [step4]
            for i in range(11):
                m_i = [jnp.broadcast_to(mul[slot, 4 * i + 2 * half + part, c:c + 1, :], (8, 128)) for part in range(2)]
                grp.append(_cmul(step4 if i < 7 else step8, m_i))
            rhs = jnp.concatenate([jnp.concatenate([v[part] for v in grp], axis=0) for part in range(2)], axis=1)
            rhs, lhs = pad_rows(rhs, 128), jnp.concatenate(lhs, axis=1)
            t = lax.dot_general(lhs, rhs, NT_DIMS, preferred_element_type=F32)
            taps = t if taps is None else taps + t
        kbuf[g // 4, PST * (8 * j + c):PST * (8 * j + c) + 8, :] = taps

    def pack_taps(i):
        lane = lax.broadcasted_iota(jnp.int32, (32, 128), 1)
        r = [kbuf[i, pl.ds(j, 32, stride=PST), :] for j in range(8)]
        x01 = jnp.where(lane < 64, r[0], pltpu.roll(r[1], 64, 1))
        x23 = jnp.where(lane < 64, r[2], pltpu.roll(r[3], 64, 1))
        t2 = jnp.where(lane < 64, r[4], pltpu.roll(r[5], 64, 1))
        packed = [
            jnp.where((lane & 32) == 0, x01, pltpu.roll(x23, 32, 1)),
            jnp.where((lane & 32) != 0, x01, pltpu.roll(x23, 96, 1)),
            jnp.where(lane == 63, r[3], t2), t2,
            jnp.where(lane == 63, r[5], r[6]), r[6],
            jnp.where(lane == 63, r[6], r[7]), r[7],
            jnp.where(lane == 63, r[7], r[3]), r[3],
            jnp.where(lane == 95, r[3], r[5]), r[5],
            jnp.where(lane == 95, r[5], r[6]),
            jnp.where(lane == 95, r[6], r[7]),
        ]
        for blk in range(NB):
            tbuf[blk, pl.ds(pl.multiple_of(i * 16, 16), 16), :] = _pack(packed[T_OF_BLOCK[blk]])
        return _token(packed[0], packed[1], packed[2])

    def taps_dft(blk, slot):
        mat = jnp.where(blk < 6, blk, jnp.where(blk < 8, blk - 2, jnp.where(blk == 8, 6, 8 - blk % 2)))
        h = jnp.dot(_unpack(tbuf[blk]), _unpack(fw_v[mat]), preferred_element_type=F32)
        h_re, h_im = h[:, :128], h[:, 128:]
        g_re, g_im = h_re + hlast[1 - slot, 0], h_im + hlast[1 - slot, 1]
        even = (lax.broadcasted_iota(jnp.int32, (D, 128), 1) & 1) == 0
        hlast[slot, 0] = jnp.where(even, -1.0, 1.0) * h_im
        hlast[slot, 1] = jnp.where(even, 1.0, -1.0) * h_re
        g_dif, g_sum = g_im - g_re, g_re + g_im
        for t, v in enumerate((g_re, g_dif, g_sum)):
            gbuf[:, 3 * blk + t] = v.reshape(D // 8, 8, 128)

    def input_dft(g, b0, nb, tokens):
        rows = pl.ds(pl.multiple_of(g * 8, 8 * GA), 8 * GA)
        u_t = jnp.concatenate([u_v[rows, b * T:(b + 1) * T] for b in range(b0, b0 + nb)], axis=0)
        r = jnp.dot(_unpack(tie(_pack(u_t), tokens)), _unpack(fw_v[9]), preferred_element_type=F32)
        for b in range(nb):
            u_re, u_im = r[8 * GA * b:8 * GA * (b + 1), :128], r[8 * GA * b:8 * GA * (b + 1), 128:]
            for t, v in enumerate((u_re + u_im, u_re, u_im)):
                ubuf[pl.ds(g, GA), 3 * (b0 + b) + t] = v.reshape(GA, 8, 128)

    def block_conv(g, k):
        rows = pl.ds(pl.multiple_of(g * 8, 8), 8)
        low = lax.broadcasted_iota(jnp.int32, (8, 128), 1) < 64
        acc, loaded = {}, {}

        def g_at(d, t):
            if (d, t) not in loaded:
                loaded[d, t] = gbuf[g, 3 * d + t]
            return loaded[d, t]

        for j in range(2 * k + 2):
            if j and j % CONV_STEP == 0:
                yield _token(acc[2 * k + 1][2])
            u_j = [ubuf[g, 3 * j + t] for t in range(3)]
            for i in range(max(j, 2 * k), 2 * k + 2):
                prod = [g_at(i - j, t) * u_j[t] for t in range(3)]
                acc[i] = [a + b for a, b in zip(acc[i], prod)] if i in acc else prod
        done = []
        for i, (k1, k2, k3) in acc.items():
            y_re, y_im = k1 - k3, k1 + k2
            swapped = pltpu.roll(jnp.where(low, y_im, y_re), 64, 1)
            first = jnp.where(low, y_re, swapped)
            second = jnp.where(low, swapped, y_im)
            done += [first + second, first - second]
            ybuf[i, 0, rows, :], ybuf[i, 1, rows, :] = done[-2:]
        yield _token(*done)

    def inverse_dft(blk, slot):
        for par in range(2):
            y = lax.dot_general(_unpack(inv_v[par]), pad_rows(ybuf[blk, par], 512).astype(BF16), NT_DIMS,
                                preferred_element_type=F32)
            for j in range(4):
                yst[slot, j, pl.ds(par, 64, stride=2), :] = y[:, 128 * j:128 * (j + 1)]
        rows = pl.ds(blk * T, T)
        for j in range(4):
            wd = min(128, D - 128 * j)
            out_v[rows, 128 * j:128 * j + wd] = yst[slot, j, :T, :].astype(BF16)[:, :wd]

    zero_ref[...] = jnp.zeros(zero_ref.shape, U32)
    for cp in first_cp:
        cp.wait()
    dtc[0] = to_column(jnp.exp(ldt_v[...].astype(F32).reshape(1, D)).astype(BF16).astype(F32))
    for cp in [x_cp(i) for i in range(4, NB)]:
        cp.start()

    @pl.loop(0, 4)
    def _(i):
        list(modes(Z0 * i, Z0))

    kbuf[0] = jnp.zeros(kbuf.shape[1:], F32)
    for cp in weight_cp:
        cp.wait()
    for i, w_ref in enumerate((wk_v, wv_v)):
        wt[D // 2 + 16 * i:D // 2 + 16 * (i + 1), :] = _pack(pad_rows(w_ref[...].astype(F32), 32))
    transpose_weight(wq_v, wt)

    def prologue(i, carry):
        for j in range(4):
            x_cp(4 * i + j).wait()
        project_kv(i)
        project_q(i, list(modes(4 * Z0 + Z1 * i, Z1)))
        return carry

    for cp in second_cp:
        cp.start()
    lax.fori_loop(0, 4, prologue, 0)
    early = list(modes(4 * (Z0 + Z1), Z2))
    m, _ = step(q_window(0, 0), None, None,
                lambda c: early[c * 2 * Z2 // (NCH - 2):(c + 1) * 2 * Z2 // (NCH - 2)], [[], []])
    for cp in second_cp:
        cp.wait()
    for cp in [u_cp(i) for i in range(D // 32)] + late_cp:
        cp.start()
    dtc[1] = to_column(dsk_v[...].astype(F32).reshape(1, D))

    def spread(streams, lag=2):
        span = 2 * NCH - lag

        def fill(c):
            out = []
            for gen, count in streams:
                count = span if count is None else count
                if c < span:
                    out += [next(gen) for _ in range((c + 1) * count // span - c * count // span)]
                if c == span - 1 and count != span:
                    assert next(gen, fill) is fill
            return [t for t in out if t is not None]
        return fill

    def once(job, at, lag=0):
        def gen():
            yield from [None] * at
            done = job()
            yield from [None] * lag + [done] + [None] * (2 * NCH)
        return gen(), None

    last_group = D // 8 - 1
    n_a = -(-(D // 8) // GA)
    n_c = -(-(D // 8) // GC)

    def phase_p(it, m):
        ahead = chain(*(powers(2 * it + j, 2 * it + j) for j in range(2)))
        n = (D // 8 - 4 * (Z0 + Z1) - Z2) // 2
        streams = [(ahead, 2 * (1 + len(POWER_PLAN))), (modes(D // 8 - n * (2 - it), n), 2 * n)]
        return head_pair(it, m, spread(streams, LAG_P), LAG_P)

    m = lax.fori_loop(0, 2, phase_p, m)

    def phase_a(it, m, query=True, more=True):
        u_cp(it).wait()
        cur, nxt = (it % 2) * GA, (1 - it % 2) * GA
        taps = (kernel_channel(GA * it + j, j, cur + j, c) for j in range(GA) for c in range(8))
        ahead = chain(*(powers(jnp.minimum(GA * (it + 1) + j, D // 8 - PW), nxt + j) for j in range(0, GA, PW)))

        def take(n):
            return [next(ahead) for _ in range(n if more else 0)]

        n_tok = (1 + len(POWER_PLAN)) * GA // PW - UP * NU
        streams = [once(lambda: pack_taps(jnp.maximum(it - 1, 0)), KP_AT, KP_LAG)]
        if query:
            streams.append(once(lambda: project_q(jnp.minimum(4 + it, NB - 1), take(NQ)), QP))
        else:
            streams.append(once(lambda: transpose_weight(wo_v, wot, (0, 1) if more else (2, 3)), WO_AT, 6))
        streams += [(taps, 8 * GA), ((input_dft(GA * it, b, NB // UP, take(NU)) for b in range(0, NB, NB // UP)), UP)]
        if more:
            streams.append((ahead, n_tok - (NQ if query else 0)))
        m = head_pair(2 + it, m, spread(streams, LAG_A), LAG_A)
        return m

    m = lax.fori_loop(0, n_a - PEEL, phase_a, m)
    for cp in late_cp:
        cp.wait()
    for it in range(n_a - PEEL, n_a):
        m = phase_a(it, m, query=False, more=it + 1 < n_a)
    pack_taps(n_a - 1)
    hlast[1, 0] = k0c[...]
    hlast[1, 1] = jnp.zeros((D, 128), F32)

    def phase_b(it, m):
        return head_pair(16 + it, m, spread([((taps_dft(8 * it + j, j % 2) for j in range(8)), 8)]))

    m = lax.fori_loop(0, 2, phase_b, m)

    def phase_c(it, m):
        convs = chain(*(block_conv(jnp.minimum(GC * it + j, last_group), k)
                        for j in range(GC) for k in range(8)))
        count = GC * sum(1 + (2 * k + 1) // CONV_STEP for k in range(8))
        proj = once(lambda: put_out(it, out_features(it, 0, D, [next(convs) for _ in range(NO)])), OP, OL)
        return head_pair(18 + it, m, spread([proj, (convs, count - NO)], LAG_C), LAG_C)

    m = lax.fori_loop(0, n_c, phase_c, m)

    def out_cp(i, rows, cols):
        return pltpu.make_async_copy(out_v.at[rows, cols], out_hbm.at[0, rows, cols], out_sem.at[i])

    done_cp = [out_cp(0, pl.ds(0, 3 * W), pl.ds(512, 384))]
    done_cp[0].start()
    m = head_pair(30, m, spread([((inverse_dft(blk, blk % YS) for blk in range(NB)), NB)]))
    done_cp += [out_cp(1, pl.ds(0, 3 * W), pl.ds(0, 512)), out_cp(2, pl.ds(3 * W, W), pl.ds(0, 384))]
    for cp in done_cp[1:]:
        cp.start()

    def fill_last(c):
        if c in LAST_AT:
            j = LAST_AT.index(c)
            qt[j] = out_features(12 + j, 0, 384)
        return []

    head_pair(31, m, fill_last, last=True)
    tails = [qt[j] + out_features(12 + j, 384, D) for j in range(W // T)]
    for j, r in enumerate(tails):
        put_out(12 + j, r)
        done_cp.append(out_cp(3 + j, pl.ds(3 * W + T * j, T), pl.ds(384, 512)))
        done_cp[-1].start()
    for cp in done_cp:
        cp.wait()


@jax.jit
def pallas_concat_heads__ssm_conv_s4__grouped_kv_mqa__prompt_kernel(
    A_u: jax.Array,
    A_A_re: jax.Array,
    A_A_im: jax.Array,
    A_B_re: jax.Array,
    A_B_im: jax.Array,
    A_C_re: jax.Array,
    A_C_im: jax.Array,
    A_log_dt: jax.Array,
    A_Dskip: jax.Array,
    B_x: jax.Array,
    B_wq: jax.Array,
    B_wk: jax.Array,
    B_wv: jax.Array,
    B_wo: jax.Array,
):
    hbm = pl.BlockSpec(memory_space=pltpu.MemorySpace.HBM)
    scratch = [
        pltpu.VMEM((D, L), BF16),
        pltpu.VMEM((6, D, N), BF16),
        pltpu.VMEM((D,), BF16),
        pltpu.VMEM((D,), BF16),
        pltpu.VMEM((NB, D, T), BF16),
        pltpu.VMEM((D, D), BF16),
        pltpu.VMEM((DH, D), BF16),
        pltpu.VMEM((DH, D), BF16),
        pltpu.VMEM((D, D), BF16),
        pltpu.VMEM((10, 64, 256), U32),
        pltpu.VMEM((2, 32, 128), U32),
        pltpu.VMEM((L, 2 * D), BF16),
        pltpu.VMEM((256, D), U32),
        pltpu.VMEM((D // 2, D), U32),
        pltpu.VMEM((NB, D, T), F32),
        pltpu.VMEM((L // 2, 128), U32),
        pltpu.VMEM((2, 16, L), U32),
        pltpu.VMEM((L, W), F32),
        pltpu.VMEM((NB, D, T), F32),
        pltpu.VMEM((2, 512, 128), F32),
        pltpu.VMEM((D, 128), F32),
        pltpu.VMEM((2, D, N), F32),
        pltpu.VMEM((2 * GA, 12, 88, 128), F32),
        pltpu.VMEM((2 * GA, 44, 8, 128), F32),
        pltpu.VMEM((D // 32, 304, 128), F32),
        pltpu.VMEM((NB, D // 2, 128), U32),
        pltpu.VMEM((2, 2, D, 128), F32),
        pltpu.VMEM((D // 8, 3 * NB, 8, 128), F32),
        pltpu.VMEM((32, 128), U32),
        pltpu.VMEM((D // 8, 3 * NB, 8, 128), F32),
        pltpu.VMEM((NB, 2, D, 128), F32),
        pltpu.VMEM((YS, 4, T + 8, 128), F32),
        pltpu.SemaphoreType.DMA((NB,)),
        pltpu.SemaphoreType.DMA((D // 32,)),
        pltpu.SemaphoreType.DMA((15,)),
        pltpu.SemaphoreType.DMA((7,)),
    ]
    return pl.pallas_call(
        _kernel,
        out_shape=jax.ShapeDtypeStruct((1, L, 2 * D), BF16),
        in_specs=[hbm] * 16,
        out_specs=hbm,
        scratch_shapes=scratch,
        compiler_params=pltpu.CompilerParams(vmem_limit_bytes=100 * 2**20),
    )(A_u.transpose(0, 2, 1), A_A_re, A_A_im, A_B_re, A_B_im, A_C_re, A_C_im, A_log_dt, A_Dskip,
      B_x.transpose(0, 2, 1), B_wq, B_wk.T, B_wv.T, B_wo, _FWD, _INV)
```
